```python
import jax
import jax.numpy as jnp

def _softmax(x, axis=-1):
    return jax.nn.softmax(x, axis=axis)
def _gelu(x):
    return jax.nn.gelu(x, approximate=True)
def _silu(x):
    return jax.nn.silu(x)
def _sigmoid(x):
    return jax.nn.sigmoid(x)
def _layernorm(x, axis=-1, eps=1e-5):
    m = jnp.mean(x, axis=axis, keepdims=True)
    v = jnp.var(x, axis=axis, keepdims=True)
    return (x - m) / jnp.sqrt(v + eps)
def _scatter_add(tgt, idx, src, axis=0):
    return tgt.at[idx].add(src)
def _segment_sum(src, seg, n):
    return jax.ops.segment_sum(src, seg, n)
class _Rng:
    def __init__(self, key):
        self._k = key
    def _next(self):
        self._k, sub = jax.random.split(self._k)
        return sub
    def normal(self, shape):
        return jax.random.normal(self._next(), shape, dtype=jnp.bfloat16)
    def randint(self, lo, hi, shape):
        return jax.random.randint(self._next(), shape, lo, hi, dtype=jnp.int32)
    def uniform(self, shape, lo=0.0, hi=1.0):
        return jax.random.uniform(self._next(), shape, jnp.bfloat16, lo, hi)
    def permutation(self, n):
        return jax.random.permutation(self._next(), n)


kernel_name = 'parallel_sum__sliding_local_dilated__mixer_token_mlp__prompt'

def setup_inputs():
    _rng = _Rng(jax.random.key(int.from_bytes(__import__("os").urandom(4), "little")))
    _w = (lambda a: (lambda t: t.astype(jnp.bfloat16) if jnp.issubdtype(t.dtype, jnp.floating) else t)(jnp.asarray(a)))
    def _A_setup():
        B, S, D = 1, 2048, 448
        return {
            "x": _w((lambda *s: _rng.normal(s) * 0.05)(B, S, D)),
            "wqkv": _w((lambda *s: _rng.normal(s) * 0.05)(D, 3 * D)),
            "wo": _w((lambda *s: _rng.normal(s) * 0.05)(D, D)),
        }
    _A_in = _A_setup()

    def _B_setup():
        B, S, D, F = 1, 2048, 448, 1792
        return {
            "x": _w((lambda *s: _rng.normal(s) * 0.05)(B, S, D)),
            "w1": _w((lambda *s: _rng.normal(s) * 0.05)(S, F) * (S ** -0.5)),
            "b1": _w((lambda *s: _rng.normal(s) * 0.05)(F) * 0.02),
            "w2": _w((lambda *s: _rng.normal(s) * 0.05)(F, S) * (F ** -0.5)),
            "b2": _w((lambda *s: _rng.normal(s) * 0.05)(S) * 0.02),
        }
    _B_in = _B_setup()

    return {
        "A_x": _A_in["x"],
        "A_wqkv": _A_in["wqkv"],
        "A_wo": _A_in["wo"],
        "B_x": _B_in["x"],
        "B_w1": _B_in["w1"],
        "B_b1": _B_in["b1"],
        "B_w2": _B_in["w2"],
        "B_b2": _B_in["b2"],
    }

def reference(A_x, A_wqkv, A_wo, B_x, B_w1, B_b1, B_w2, B_b2):
    def _A_ref(x, wqkv, wo):
        B, S, D = x.shape
        H = 16; Dh = D // H
        W, dil = 8, 2
        qkv = (lambda x, *d: x.transpose(*d))((x @ wqkv).reshape(B, S, 3, H, Dh), 2, 0, 3, 1, 4)
        q, k, v = qkv[0], qkv[1], qkv[2]
        scale = Dh ** -0.5
        pos = jnp.arange(S)
        off = jnp.arange(W) * dil
        idx = pos[:, None] - off[None, :]
        mask = idx >= 0
        idx_c = jnp.where(mask, idx, 0).reshape(-1)
        kg = k[:, :, idx_c, :].reshape(B, H, S, W, Dh)
        vg = v[:, :, idx_c, :].reshape(B, H, S, W, Dh)
        logits = jnp.einsum("bhsd,bhswd->bhsw", q, kg) * scale
        logits = jnp.where(mask[None, None, :, :], logits, -1e9)
        attn = _softmax(logits, axis=-1)
        o = jnp.einsum("bhsw,bhswd->bhsd", attn, vg)
        return (lambda x, *d: x.transpose(*d))(o, 0, 2, 1, 3).reshape(B, S, D) @ wo

    def _B_ref(x, w1, b1, w2, b2):
        B, S, D = x.shape
        h = _layernorm(x, axis=-1)
        u = jnp.einsum("bsd,sf->bdf", h, w1) + b1
        u = _gelu(u)
        y = jnp.einsum("bdf,fs->bds", u, w2) + b2
        return (lambda x, *d: x.transpose(*d))(y, 0, 2, 1)

    x = A_x
    xn = _layernorm(x, axis=-1)
    return x + _A_ref(xn, A_wqkv, A_wo) + _B_ref(xn, B_w1, B_b1, B_w2, B_b2)
```

```python
import math

import jax
import jax.numpy as jnp
import numpy as np
from jax import lax
from jax.experimental import pallas as pl
from jax.experimental.pallas import tpu as pltpu

F32 = jnp.float32
BF16 = jnp.bfloat16
U32 = jnp.uint32

H = 16
W = 8
DIL = 2
LANES = 128
EPS = 1e-5

T1 = 256
N2 = 256
N3 = 256
N4 = 256

_NT = (((1,), (1,)), ((), ()))
_GELU_C = math.sqrt(2.0 / math.pi)


def _lane_splits(n):
    return [(s, min(LANES, n - s)) for s in range(0, n, LANES)]


def _ds(start, size, align=None):
    if isinstance(start, int):
        return pl.ds(start, size)
    return pl.ds(pl.multiple_of(start, align or size), size)


def _layernorm_cols(x):
    m = jnp.mean(x, axis=0, keepdims=True)
    xc = x - m
    v = jnp.mean(xc * xc, axis=0, keepdims=True)
    return xc * lax.rsqrt(v + EPS)


def _gelu(u):
    inner = _GELU_C * (u + 0.044715 * (u * u * u))
    return 0.5 * u * (1.0 + jnp.tanh(inner))


def _kernel(
    x_hbm, wqkv_hbm, wo_hbm, w1_hbm, w2_hbm,
    b1_ref, b2_ref,
    out_hbm,
    x_v, wqkv_v, wo_v, w1_v, w2_v,
    wqkv_t, wo_f, wo_p, wo_t,
    h_v, xn_tok, u_v, g_v,
    q_v, k_v, v_v, o_tok, y_v, b2_v, out_v,
    sem_x, sem_w1, sem_w2, sem_qkv, sem_wo, sem_out,
    *, S, D, F,
):
    DH = D // H
    NT = S // LANES
    C1, C2, C3, C4 = S // T1, S // N2, S // N3, S // N4
    HALO = W - 1
    scale = DH ** -0.5
    dsplits = _lane_splits(D)

    def cp_x(c):
        sl = _ds(c * T1, T1)
        return pltpu.make_async_copy(x_hbm.at[:, sl], x_v.at[:, sl], sem_x.at[c])

    def cp_w1(c):
        return pltpu.make_async_copy(
            w1_hbm.at[_ds(c * T1, T1), :], w1_v.at[c], sem_w1.at[c])

    def cp_w2(c):
        return pltpu.make_async_copy(
            w2_hbm.at[:, _ds(c * N3, N3)], w2_v.at[c], sem_w2.at[c])

    def cp_out(c):
        return pltpu.make_async_copy(
            out_v.at[c], out_hbm.at[:, _ds(c * N4, N4)], sem_out.at[c])

    cp_wqkv = pltpu.make_async_copy(wqkv_hbm, wqkv_v, sem_qkv)
    cp_wo = pltpu.make_async_copy(wo_hbm, wo_v, sem_wo)

    for c in range(C1):
        cp_x(c).start()
        cp_w1(c).start()
    cp_wqkv.start()
    cp_wo.start()

    b1 = b1_ref[...].astype(F32).reshape(1, F)
    u_v[...] = jnp.broadcast_to(b1, (D, F))
    s_last, w_last = dsplits[-1]
    if w_last < LANES:
        xn_tok[len(dsplits) - 1] = jnp.zeros((S // 2, LANES), U32)
        o_tok[len(dsplits) - 1] = jnp.zeros((S // 2, LANES), U32)
        wo_f[len(dsplits) - 1] = jnp.zeros((D, LANES), F32)

    def norms(c):
        sl = _ds(c * T1, T1)
        xn = _layernorm_cols(x_v[:, sl].astype(F32))
        h_v[:, sl] = _layernorm_cols(xn).astype(BF16)
        words = pltpu.bitcast(xn.astype(BF16).T, U32)
        rows = _ds(c * (T1 // 2), T1 // 2)
        for i, (s0, w) in enumerate(dsplits):
            xn_tok[i, rows, 0:w] = words[:, s0:s0 + w]

    def mix1(c):
        sl = _ds(c * T1, T1)
        u_v[...] += jnp.dot(h_v[:, sl], w1_v[c], preferred_element_type=F32)

    cp_x(0).wait()
    norms(0)

    def p1_body(c, carry):
        cp_w1(c).wait()
        cp_x(c + 1).wait()
        mix1(c)
        norms(c + 1)
        return carry

    lax.fori_loop(0, C1 - 1, p1_body, 0)

    for c in range(C3):
        cp_w2(c).start()

    cp_w1(C1 - 1).wait()
    cp_wqkv.wait()
    cp_wo.wait()
    mix1(C1 - 1)
    wqkv_t[...] = wqkv_v[...].T
    for i, (s0, w) in enumerate(dsplits):
        wo_f[i, :, 0:w] = wo_v[:, s0:s0 + w].astype(F32)
    for d in range(DH):
        rows = [wo_f[i, pl.ds(d, H, stride=DH), :][:, 0:w] for i, (s0, w) in enumerate(dsplits)]
        wo_p[d * H:(d + 1) * H, :] = jnp.concatenate(rows, axis=1).astype(BF16)
    wo_t[...] = wo_p[...].T

    P2 = N2 // LANES
    FG = -(-(F // LANES) // C2) * LANES

    def qkv(c):
        tiles = []
        for p in range(P2):
            j = c * P2 + p
            cols = [
                pltpu.bitcast(xn_tok[i, pl.ds(j, LANES // 2, stride=NT), :], BF16)[:, 0:w]
                for i, (s0, w) in enumerate(dsplits)
            ]
            tiles.append(jnp.concatenate(cols, axis=1))
        rows = jnp.concatenate(tiles, axis=0)
        r = lax.dot_general(wqkv_t[...], rows, _NT, preferred_element_type=F32)
        for p in range(P2):
            j = c * P2 + p
            ls = slice(p * LANES, (p + 1) * LANES)
            q_v[j] = r[0:D, ls]
            k_v[j + HALO] = r[D:2 * D, ls]
            v_v[j + HALO] = r[2 * D:3 * D, ls]

    def gelu_cols(f0, width):
        sl = _ds(f0, width, LANES)
        g_v[:, sl] = _gelu(u_v[:, sl]).astype(BF16)

    n_g = F // FG

    def p2_body(c, carry):
        qkv(c)
        gelu_cols(c * FG, FG)
        return carry

    lax.fori_loop(0, n_g, p2_body, 0)
    for c in range(n_g, C2):
        qkv(c)
        if c == n_g and F > n_g * FG:
            gelu_cols(n_g * FG, F - n_g * FG)

    def halo_body(i, carry):
        k_v[i] = pltpu.roll(k_v[i + NT], DIL, 1)
        v_v[i] = pltpu.roll(v_v[i + NT], DIL, 1)
        return carry

    lax.fori_loop(0, HALO, halo_body, 0)

    P3 = N3 // LANES
    lane = lax.broadcasted_iota(jnp.int32, (H, LANES), 1)

    def attend(j):
        def head_rows(ref, t, d):
            return ref[t, pl.ds(d, H, stride=DH), :]

        logit = [None] * W
        for d in range(DH):
            qd = head_rows(q_v, j, d)
            for w in range(W):
                t = qd * head_rows(k_v, j + HALO - w, d)
                logit[w] = t if logit[w] is None else logit[w] + t
        for w in range(W):
            lw = logit[w] * scale
            if w > 0:
                lw = jnp.where((lane < DIL) & (j < w), -1e9, lw)
            logit[w] = lw
        mx = logit[0]
        for w in range(1, W):
            mx = jnp.maximum(mx, logit[w])
        e = [jnp.exp(logit[w] - mx) for w in range(W)]
        den = e[0]
        for w in range(1, W):
            den = den + e[w]
        inv = 1.0 / den
        p = [e[w] * inv for w in range(W)]
        outs = []
        for d in range(DH):
            acc = None
            for w in range(W):
                t = p[w] * head_rows(v_v, j + HALO - w, d)
                acc = t if acc is None else acc + t
            outs.append(acc.astype(BF16))
        o = jnp.concatenate(outs, axis=0)
        words = pltpu.bitcast(o.T, U32)
        for i, (s0, w) in enumerate(dsplits):
            o_tok[i, pl.ds(j, LANES // 2, stride=NT), 0:w] = words[:, s0:s0 + w]

    def p3_body(c, carry):
        cp_w2(c).wait()
        sl = _ds(c * N3, N3)
        y_v[:, sl] = jnp.dot(g_v[...], w2_v[c], preferred_element_type=F32)
        for p in range(P3):
            attend(c * P3 + p)
        return carry

    lax.fori_loop(0, C3, p3_body, 0)

    b2_v[...] = b2_ref[...].astype(F32).reshape(1, S)

    def p4_body(c, carry):
        sl = _ds(c * N4, N4)
        rows = _ds(c * (N4 // 2), N4 // 2)
        cols = [
            pltpu.bitcast(o_tok[i, rows, :], BF16)[:, 0:w] for i, (s0, w) in enumerate(dsplits)
        ]
        o = jnp.concatenate(cols, axis=1)
        a = lax.dot_general(wo_t[...], o, _NT, preferred_element_type=F32)
        res = x_v[:, sl].astype(F32) + a + (y_v[:, sl] + b2_v[:, sl])
        out_v[c] = res.astype(BF16)
        cp_out(c).start()
        return carry

    for c in range(C4):
        p4_body(c, 0)
    for c in range(C4):
        cp_out(c).wait()


@jax.jit
def pallas_parallel_sum__sliding_local_dilated__mixer_token_mlp__prompt_kernel(
    A_x: jax.Array,
    A_wqkv: jax.Array,
    A_wo: jax.Array,
    B_x: jax.Array,
    B_w1: jax.Array,
    B_b1: jax.Array,
    B_w2: jax.Array,
    B_b2: jax.Array,
):
    del B_x
    Bsz, S, D = A_x.shape
    F = B_w1.shape[1]
    assert Bsz == 1 and S == 16 * LANES and D % H == 0 and D % 16 == 0
    assert F % LANES == 0
    nct = -(-D // LANES)
    NT = S // LANES
    HALO = W - 1

    x_t = A_x.reshape(S, D).T

    def kern(*refs):
        _kernel(*refs, S=S, D=D, F=F)

    hbm = pl.BlockSpec(memory_space=pl.ANY)
    vmem = pl.BlockSpec(memory_space=pltpu.VMEM)
    scratch = [
        pltpu.VMEM((D, S), BF16),
        pltpu.VMEM((D, 3 * D), BF16),
        pltpu.VMEM((D, D), BF16),
        pltpu.VMEM((S // T1, T1, F), BF16),
        pltpu.VMEM((S // N3, F, N3), BF16),
        pltpu.VMEM((3 * D, D), BF16),
        pltpu.VMEM((nct, D, LANES), F32),
        pltpu.VMEM((D, D), BF16),
        pltpu.VMEM((D, D), BF16),
        pltpu.VMEM((D, S), BF16),
        pltpu.VMEM((nct, S // 2, LANES), U32),
        pltpu.VMEM((D, F), F32),
        pltpu.VMEM((D, F), BF16),
        pltpu.VMEM((NT, D, LANES), F32),
        pltpu.VMEM((NT + HALO, D, LANES), F32),
        pltpu.VMEM((NT + HALO, D, LANES), F32),
        pltpu.VMEM((nct, S // 2, LANES), U32),
        pltpu.VMEM((D, S), F32),
        pltpu.VMEM((1, S), F32),
        pltpu.VMEM((S // N4, D, N4), BF16),
        pltpu.SemaphoreType.DMA((S // T1,)),
        pltpu.SemaphoreType.DMA((S // T1,)),
        pltpu.SemaphoreType.DMA((S // N3,)),
        pltpu.SemaphoreType.DMA(()),
        pltpu.SemaphoreType.DMA(()),
        pltpu.SemaphoreType.DMA((S // N4,)),
    ]
    out_t = pl.pallas_call(
        kern,
        out_shape=jax.ShapeDtypeStruct((D, S), BF16),
        in_specs=[hbm, hbm, hbm, hbm, hbm, vmem, vmem],
        out_specs=hbm,
        scratch_shapes=scratch,
        compiler_params=pltpu.CompilerParams(vmem_limit_bytes=100 * 1024 * 1024),
    )(x_t, A_wqkv, A_wo, B_w1, B_w2, B_b1, B_b2)
    return out_t.T.reshape(1, S, D)
```

```python
import math

import jax
import jax.numpy as jnp
from jax import lax
from jax.experimental import pallas as pl
from jax.experimental.pallas import tpu as pltpu

F32 = jnp.float32
BF16 = jnp.bfloat16
U32 = jnp.uint32

H = 16
W = 8
DIL = 2
LANES = 128
SUB = 8
RG = 16
EPS = 1e-5

P1_CHUNKS = (256, 256, 256, 256, 256, 256, 256, 256)
OUT_CHUNKS = (256, 256, 256, 256, 256, 256, 256, 128, 128)
TIES = True
ATT_TILES = 14
TOK_PITCH = 18
ATT_PITCH = 66

_NN = (((1,), (0,)), ((), ()))
_NT = (((1,), (1,)), ((), ()))
_GELU_C = math.sqrt(2.0 / math.pi)


def _lane_splits(n):
    return [(s, min(LANES, n - s)) for s in range(0, n, LANES)]


def _words(v):
    return pltpu.bitcast(v.astype(BF16), U32)


def _halves(w):
    return pltpu.bitcast(w, BF16)


def _bits(v):
    return pltpu.bitcast(jnp.broadcast_to(v, (SUB, LANES)), U32)


def _gelu(u):
    inner = _GELU_C * (u + 0.044715 * (u * u * u))
    return 0.5 * u * (1.0 + jnp.tanh(inner))


def _col_mean(v):
    acc = v[0:SUB]
    for i in range(1, v.shape[0] // SUB):
        acc = acc + v[i * SUB:(i + 1) * SUB]
    return jnp.sum(acc, axis=0, keepdims=True) / v.shape[0]


class _Schedule:
    def __init__(self):
        self.zero = None
        self.plan = {}

    def spread(self, jobs, slots):
        total = sum(c for c, _ in jobs)
        done = 0
        for cost, fn in jobs:
            done += cost
            unit, rg = slots[min(len(slots) - 1, (done * len(slots) - 1) // total)]
            self.plan.setdefault(unit, []).append((rg, fn))

    def operand(self, unit, load, n_rg):
        tokens = {}
        for rg, fn in self.plan.pop(unit, []):
            for t in fn() or []:
                tokens[rg] = t if rg not in tokens else tokens[rg] | t
        if not TIES:
            tokens = {}
        parts, start = [], 0
        for rg in sorted(tokens):
            if rg > start:
                parts.append(load(start * SUB, rg * SUB))
            blk = load(rg * SUB, (rg + 1) * SUB)
            head = blk[:, :LANES] | (tokens[rg] & self.zero)
            parts.append(head if blk.shape[1] == LANES else jnp.concatenate([head, blk[:, LANES:]], axis=1))
            start = rg + 1
        if start < n_rg:
            parts.append(load(start * SUB, n_rg * SUB))
        return _halves(parts[0] if len(parts) == 1 else jnp.concatenate(parts, axis=0))


def _kernel(
    x_hbm, wqkv_hbm, wo_hbm, w1_hbm, w2_hbm, b1_hbm, b2_hbm,
    out_hbm,
    x_v, wqkv_v, wo_v, w1_v, w2_v, b1_v, b2_v, zero_src, zero_v,
    wqkv_w, wo_f, wo_p, wo_w,
    xn_f, xn_w, h_w, xn_tok, u_f, g_w,
    q_f, k_f, v_f, o_w, o_tok, y_f, out_v,
    sem_x, sem_w1, sem_misc, sem_out,
    *, S, D, F,
):
    DH = D // H
    NT = S // LANES
    NF = F // LANES
    HALO = W - 1
    DW = D // 2
    D_RG = D // RG
    scale = DH ** -0.5
    dsplits = _lane_splits(D)
    sched = _Schedule()

    starts1 = [sum(P1_CHUNKS[:c]) for c in range(len(P1_CHUNKS))]
    cp_x = [
        pltpu.make_async_copy(x_hbm.at[:, s0:s0 + n], x_v.at[:, s0:s0 + n], sem_x.at[c])
        for c, (s0, n) in enumerate(zip(starts1, P1_CHUNKS))
    ]
    cp_w1 = [
        pltpu.make_async_copy(w1_hbm.at[s0:s0 + n, :], w1_v.at[s0:s0 + n, :], sem_w1.at[c])
        for c, (s0, n) in enumerate(zip(starts1, P1_CHUNKS))
    ]
    cp_b1 = pltpu.make_async_copy(b1_hbm, b1_v, sem_misc.at[0])
    cp_b2 = pltpu.make_async_copy(b2_hbm, b2_v, sem_misc.at[1])
    cp_wqkv = pltpu.make_async_copy(wqkv_hbm, wqkv_v, sem_misc.at[2])
    cp_wo = pltpu.make_async_copy(wo_hbm, wo_v, sem_misc.at[3])
    cp_w2 = pltpu.make_async_copy(w2_hbm, w2_v, sem_misc.at[4])
    cp_zero = pltpu.make_async_copy(zero_src, zero_v, sem_misc.at[5])
    starts_out = [sum(OUT_CHUNKS[:c]) for c in range(len(OUT_CHUNKS))]
    cp_out = [
        pltpu.make_async_copy(out_v.at[:, s0:s0 + n], out_hbm.at[:, s0:s0 + n], sem_out.at[c])
        for c, (s0, n) in enumerate(zip(starts_out, OUT_CHUNKS))
    ]

    cp_x[0].start()
    cp_w1[0].start()
    cp_b1.start()
    zero_src[...] = jnp.zeros((SUB, LANES), U32)
    cp_zero.start()
    for c in range(1, len(P1_CHUNKS)):
        cp_x[c].start()
        cp_w1[c].start()
    cp_wqkv.start()
    cp_wo.start()
    cp_b2.start()
    cp_w2.start()

    def norm_jobs(t):
        ls = slice(t * LANES, (t + 1) * LANES)
        st = {}

        def mean1():
            st["m"] = _col_mean(x_v[:, ls].astype(F32))
            return [_bits(st["m"])]

        def var1():
            xc = x_v[:, ls].astype(F32) - st["m"]
            st["r"] = lax.rsqrt(_col_mean(xc * xc) + EPS)
            return [_bits(st["r"])]

        def apply1():
            xn = (x_v[:, ls].astype(F32) - st["m"]) * st["r"]
            xn_f[t] = xn
            xn_w[t] = _words(xn)
            st["m2"] = _col_mean(xn)
            return [_bits(st["m2"])]

        def transpose(i):
            def job():
                s0, w = dsplits[i]
                tw = pltpu.bitcast(_halves(xn_w[t, s0 // 2:(s0 + w) // 2, :]).T, U32)
                for q in range(4):
                    r0 = (4 * t + q) * TOK_PITCH
                    xn_tok[i, r0:r0 + NT, 0:w] = tw[q * NT:(q + 1) * NT]
                return [tw[-SUB:]] if w == LANES else []
            return job

        def var2():
            xc = xn_f[t] - st["m2"]
            st["r2"] = lax.rsqrt(_col_mean(xc * xc) + EPS)
            return [_bits(st["r2"])]

        def apply2(a, b):
            def job():
                hw = _words((xn_f[t, a * RG:b * RG, :] - st["m2"]) * st["r2"])
                h_w[a * SUB:b * SUB, ls] = hw
                return [hw[i * SUB:(i + 1) * SUB] for i in range(b - a)]
            return job

        q = D_RG // 4
        return ([(4, mean1), (7, var1), (9, apply1)] + [(1, transpose(i)) for i in range(len(dsplits))]
                + [(6, var2)] + [(2, apply2(i * q, (i + 1) * q)) for i in range(4)])

    def wqkv_jobs():
        def tile(i, o0, ow):
            def job():
                s0, w = dsplits[i]
                tw = pltpu.bitcast(wqkv_v[s0:s0 + w, o0:o0 + ow].T, U32)
                wqkv_w[o0 // 2:(o0 + ow) // 2, s0:s0 + w] = tw
                return [tw[-SUB:]] if w == LANES else []
            return job
        return [(1, tile(i, o0, ow)) for o0, ow in _lane_splits(3 * D) for i in range(len(dsplits))]

    def wo_jobs():
        def widen(i):
            def job():
                s0, w = dsplits[i]
                v = wo_v[:, s0:s0 + w].astype(F32)
                wo_f[i, :, 0:w] = v
                return [_bits(v[-SUB:])] if w == LANES else []
            return job

        def regroup(d):
            def job():
                rows = [wo_f[i, pl.ds(d, H, stride=DH), :][:, 0:w] for i, (s0, w) in enumerate(dsplits)]
                pw = _words(jnp.concatenate(rows, axis=1))
                wo_p[d * SUB:(d + 1) * SUB, :] = pw
                return [pw[:, :LANES]]
            return job

        def turn(i, o0, ow):
            def job():
                s0, w = dsplits[i]
                tw = pltpu.bitcast(_halves(wo_p[s0 // 2:(s0 + w) // 2, o0:o0 + ow]).T, U32)
                wo_w[o0 // 2:(o0 + ow) // 2, s0:s0 + w] = tw
                return [tw[-SUB:]] if w == LANES else []
            return job

        return ([(2, widen(i)) for i in range(len(dsplits))] + [(1, regroup(d)) for d in range(DH)]
                + [(1, turn(i, o0, ow)) for i in range(len(dsplits)) for o0, ow in dsplits])

    units1 = []
    for c, n in enumerate(P1_CHUNKS):
        step = max(LANES, 4 * LANES * LANES // n)
        units1 += [(c, n0, min(step, F - n0)) for n0 in range(0, F, step)]
    first_unit = {c: min(i for i, u in enumerate(units1) if u[0] == c) for c in range(len(P1_CHUNKS))}
    count = {c: sum(1 for u in units1 if u[0] == c) for c in range(len(P1_CHUNKS))}

    def slots1(c):
        return [(("p1", first_unit[c] + i), rg) for i in range(count[c]) for rg in range(D_RG)]

    last = len(P1_CHUNKS) - 1
    for c in range(last):
        t0 = starts1[c + 1] // LANES
        jobs = []
        for t in range(t0, t0 + P1_CHUNKS[c + 1] // LANES):
            jobs += norm_jobs(t)
        sched.spread(jobs, slots1(c))
    sched.spread(wqkv_jobs(), slots1(last))

    cp_x[0].wait()
    for t in range(P1_CHUNKS[0] // LANES):
        for _, job in norm_jobs(t):
            job()
    cp_b1.wait()
    cp_zero.wait()
    sched.zero = zero_v[...]
    b1 = b1_v[...].astype(F32).reshape(1, F)

    for i, (c, n0, width) in enumerate(units1):
        s0, n = starts1[c], P1_CHUNKS[c]
        if i == first_unit[c]:
            cp_w1[c].wait()
            if c < last:
                cp_x[c + 1].wait()
            else:
                cp_wqkv.wait()
        lhs = sched.operand(("p1", i), lambda a, b: h_w[a:b, s0:s0 + n], D_RG)
        r = lax.dot_general(lhs, w1_v[s0:s0 + n, n0:n0 + width], _NN, preferred_element_type=F32)
        if c == 0:
            u_f[:, n0:n0 + width] = r + b1[:, n0:n0 + width]
        else:
            u_f[:, n0:n0 + width] += r

    order2 = list(range(NT - HALO, NT)) + list(range(NT - HALO))

    def gelu_jobs(f):
        def job(rg):
            def run():
                gw = _words(_gelu(u_f[rg * RG:(rg + 1) * RG, f * LANES:(f + 1) * LANES]))
                g_w[rg * SUB:(rg + 1) * SUB, f * LANES:(f + 1) * LANES] = gw
                return [gw]
            return run
        return [(3, job(rg)) for rg in range(D_RG)]

    def halo_jobs(j):
        def job(ref, a, b):
            def run():
                r = pltpu.roll(ref[j + HALO, a:b, :], DIL, 1)
                ref[j + HALO - NT, a:b, :] = r
                return [_bits(r[i:i + SUB]) for i in range(0, b - a, 4 * SUB)]
            return run
        q = D // 4
        return [(4, job(ref, a, a + q)) for ref in (k_f, v_f) for a in range(0, D, q)]

    n_qkv_rg = 3 * D // RG
    gelu_all = [job for f in range(NF) for job in gelu_jobs(f)]
    per = -(-len(gelu_all) // 15)
    wo_prep = wo_jobs()
    for i, j in enumerate(order2):
        jobs = gelu_all[i * per:(i + 1) * per] if i < 15 else []
        if i >= 1 and order2[i - 1] >= NT - HALO:
            halo = halo_jobs(order2[i - 1])
            jobs = jobs[:len(jobs) // 2] + halo + jobs[len(jobs) // 2:]
        if i >= 9:
            k = -(-len(wo_prep) // 7)
            jobs = jobs + wo_prep[(i - 9) * k:(i - 8) * k]
        sched.spread(jobs, [(("p2", i), rg) for rg in range(n_qkv_rg)])

    cp_wo.wait()
    for i, j in enumerate(order2):
        cols = [
            _halves(xn_tok[a, pl.ds(j, LANES // 2, stride=TOK_PITCH), :])[:, 0:w]
            for a, (s0, w) in enumerate(dsplits)
        ]
        rows = jnp.concatenate(cols, axis=1)
        lhs = sched.operand(("p2", i), lambda a, b: wqkv_w[a:b, :], n_qkv_rg)
        r = lax.dot_general(lhs, rows, _NT, preferred_element_type=F32)
        q_f[j] = r[0:D]
        k_f[j + HALO] = r[D:2 * D]
        v_f[j + HALO] = r[2 * D:3 * D]

    lane = lax.broadcasted_iota(jnp.int32, (H, LANES), 1)

    def attention_jobs(j):
        st = {}

        def head_rows(ref, t, d):
            return ref[t, pl.ds(d, H, stride=DH), :]

        def logits(w):
            def job():
                acc = None
                for d in range(DH):
                    t = head_rows(q_f, j, d) * head_rows(k_f, j + HALO - w, d)
                    acc = t if acc is None else acc + t
                acc = acc * scale
                if w > j:
                    acc = jnp.where(lane < DIL, -1e9, acc)
                st[w] = acc
                return [_bits(acc[:SUB]), _bits(acc[SUB:])]
            return job

        def softmax():
            mx = st[0]
            for w in range(1, W):
                mx = jnp.maximum(mx, st[w])
            e = [jnp.exp(st[w] - mx) for w in range(W)]
            den = e[0]
            for w in range(1, W):
                den = den + e[w]
            inv = 1.0 / den
            st["p"] = [e[w] * inv for w in range(W)]
            return [_bits(p[a:a + SUB]) for p in st["p"] for a in (0, SUB)]

        def values(d):
            def job():
                acc = None
                for w in range(W):
                    t = st["p"][w] * head_rows(v_f, j + HALO - w, d)
                    acc = t if acc is None else acc + t
                ow = _words(acc)
                o_w[j, d * SUB:(d + 1) * SUB, :] = ow
                return [ow]
            return job

        def scatter(i):
            def job():
                s0, w = dsplits[i]
                tw = pltpu.bitcast(_halves(o_w[j, s0 // 2:(s0 + w) // 2, :]).T, U32)
                o_tok[i, j * ATT_PITCH:j * ATT_PITCH + LANES // 2, 0:w] = tw
                return [tw[-SUB:]] if w == LANES else []
            return job

        core = [(110, logits(w)) for w in range(W)] + [(130, softmax)]
        core += [(32, values(d)) for d in range(DH)]
        return core, [(20, scatter(i)) for i in range(len(dsplits))]

    kgroups = [(k0, min(4 * LANES, F - k0)) for k0 in range(0, F, 4 * LANES)]

    def slots3(ns):
        return [(("p3", n, g), rg) for n in ns for g, (k0, kw) in enumerate(kgroups)
                if kw == 4 * LANES for rg in range(D_RG)]

    att = [attention_jobs(j) for j in range(NT)]
    for n in range(ATT_TILES):
        lo, hi = n * NT // ATT_TILES, (n + 1) * NT // ATT_TILES
        sched.spread([job for j in range(lo, hi) for job in att[j][0]], slots3([n]))
    sched.spread([job for j in range(NT) for job in att[j][1]], slots3(range(ATT_TILES, NT)))

    cp_b2.wait()
    cp_w2.wait()
    b2 = b2_v[...].astype(F32).reshape(1, S)
    for n in range(NT):
        ls = slice(n * LANES, (n + 1) * LANES)
        for g, (k0, kw) in enumerate(kgroups):
            lhs = sched.operand(("p3", n, g), lambda a, b: g_w[a:b, k0:k0 + kw], D_RG)
            r = lax.dot_general(lhs, w2_v[k0:k0 + kw, ls], _NN, preferred_element_type=F32)
            if g == 0:
                y_f[:, ls] = r + b2[:, ls]
            else:
                y_f[:, ls] += r

    ends_out = {s0 + n: c for c, (s0, n) in enumerate(zip(starts_out, OUT_CHUNKS))}
    for n in range(NT):
        ls = slice(n * LANES, (n + 1) * LANES)
        cols = [
            jnp.concatenate(
                [_halves(o_tok[a, pl.ds(4 * n + q, NT, stride=ATT_PITCH), :]) for q in range(4)], axis=0
            )[:, 0:w]
            for a, (s0, w) in enumerate(dsplits)
        ]
        o = jnp.concatenate(cols, axis=1)
        lhs = sched.operand(("p4", n), lambda a, b: wo_w[a:b, :], D_RG)
        a = lax.dot_general(lhs, o, _NT, preferred_element_type=F32)
        out_v[:, ls] = (x_v[:, ls].astype(F32) + a + y_f[:, ls]).astype(BF16)
        if (n + 1) * LANES in ends_out:
            cp_out[ends_out[(n + 1) * LANES]].start()
    assert not sched.plan, list(sched.plan)
    for cp in cp_out:
        cp.wait()


@jax.jit
def pallas_parallel_sum__sliding_local_dilated__mixer_token_mlp__prompt_kernel(
    A_x: jax.Array,
    A_wqkv: jax.Array,
    A_wo: jax.Array,
    B_x: jax.Array,
    B_w1: jax.Array,
    B_b1: jax.Array,
    B_w2: jax.Array,
    B_b2: jax.Array,
):
    del B_x
    Bsz, S, D = A_x.shape
    F = B_w1.shape[1]
    assert Bsz == 1 and S == 16 * LANES and D % H == 0 and D % (4 * RG) == 0 and F % LANES == 0
    assert sum(P1_CHUNKS) == S and sum(OUT_CHUNKS) == S
    nct = -(-D // LANES)
    NT = S // LANES
    HALO = W - 1

    x_t = A_x.reshape(S, D).T

    def kern(*refs):
        _kernel(*refs, S=S, D=D, F=F)

    hbm = pl.BlockSpec(memory_space=pl.ANY)
    scratch = [
        pltpu.VMEM((D, S), BF16),
        pltpu.VMEM((D, 3 * D), BF16),
        pltpu.VMEM((D, D), BF16),
        pltpu.VMEM((S, F), BF16),
        pltpu.VMEM((F, S), BF16),
        pltpu.VMEM((F,), BF16),
        pltpu.VMEM((S,), BF16),
        pltpu.VMEM((SUB, LANES), U32),
        pltpu.VMEM((SUB, LANES), U32),
        pltpu.VMEM((3 * D // 2, D), U32),
        pltpu.VMEM((nct, D, LANES), F32),
        pltpu.VMEM((D // 2, D), U32),
        pltpu.VMEM((D // 2, D), U32),
        pltpu.VMEM((NT, D, LANES), F32),
        pltpu.VMEM((NT, D // 2, LANES), U32),
        pltpu.VMEM((D // 2, S), U32),
        pltpu.VMEM((nct, (S // 32) * TOK_PITCH, LANES), U32),
        pltpu.VMEM((D, F), F32),
        pltpu.VMEM((D // 2, F), U32),
        pltpu.VMEM((NT, D, LANES), F32),
        pltpu.VMEM((NT + HALO, D, LANES), F32),
        pltpu.VMEM((NT + HALO, D, LANES), F32),
        pltpu.VMEM((NT, D // 2, LANES), U32),
        pltpu.VMEM((nct, NT * ATT_PITCH, LANES), U32),
        pltpu.VMEM((D, S), F32),
        pltpu.VMEM((D, S), BF16),
        pltpu.SemaphoreType.DMA((len(P1_CHUNKS),)),
        pltpu.SemaphoreType.DMA((len(P1_CHUNKS),)),
        pltpu.SemaphoreType.DMA((6,)),
        pltpu.SemaphoreType.DMA((len(OUT_CHUNKS),)),
    ]
    out_t = pl.pallas_call(
        kern,
        out_shape=jax.ShapeDtypeStruct((D, S), BF16),
        in_specs=[hbm] * 7,
        out_specs=hbm,
        scratch_shapes=scratch,
        compiler_params=pltpu.CompilerParams(vmem_limit_bytes=100 * 1024 * 1024),
    )(x_t, A_wqkv, A_wo, B_w1, B_w2, B_b1, B_b2)
    return out_t.T.reshape(1, S, D)
```

```python
import math

import jax
import jax.numpy as jnp
from jax import lax
from jax.experimental import pallas as pl
from jax.experimental.pallas import tpu as pltpu

F32 = jnp.float32
BF16 = jnp.bfloat16
U32 = jnp.uint32

H = 16
W = 8
DIL = 2
LANES = 128
SUB = 8
RG = 16
EPS = 1e-5

T1 = 256
OUT_CHUNKS = (256, 256, 256, 256, 256, 256, 256, 128, 128)
SKEW = (0, 1, 0, 1, 2)
W1_HEAD = 768
ATT_TILES = 14
TOK_PITCH = 18
ATT_PITCH = 66

_NN = (((1,), (0,)), ((), ()))
_NT = (((1,), (1,)), ((), ()))
_GELU_C = math.sqrt(2.0 / math.pi)


def _ds(start, size, align=None):
    if isinstance(start, int):
        return pl.ds(start, size)
    return pl.ds(pl.multiple_of(start, align or size), size)


def _lane_splits(n):
    return [(s, min(LANES, n - s)) for s in range(0, n, LANES)]


def _words(v):
    return pltpu.bitcast(v.astype(BF16), U32)


def _halves(w):
    return pltpu.bitcast(w, BF16)


def _bits(v):
    return pltpu.bitcast(jnp.broadcast_to(v, (SUB, LANES)), U32)


def _gelu(u):
    inner = _GELU_C * (u + 0.044715 * (u * u * u))
    return 0.5 * u * (1.0 + jnp.tanh(inner))


def _col_mean(v):
    acc = v[0:SUB]
    for i in range(1, v.shape[0] // SUB):
        acc = acc + v[i * SUB:(i + 1) * SUB]
    return jnp.sum(acc, axis=0, keepdims=True) / v.shape[0]


class _Schedule:
    def __init__(self):
        self.zero = None
        self.plan = {}

    def spread(self, jobs, slots):
        total = sum(c for c, _ in jobs)
        done = 0
        for cost, fn in jobs:
            done += cost
            unit, rg = slots[min(len(slots) - 1, (done * len(slots) - 1) // total)]
            self.plan.setdefault(unit, []).append((rg, fn))

    def operand(self, unit, load, n_rg):
        tokens = {}
        for rg, fn in self.plan.pop(unit, []):
            for t in fn() or []:
                tokens[rg] = t if rg not in tokens else tokens[rg] | t
        parts, start = [], 0
        for rg in sorted(tokens):
            if rg > start:
                parts.append(load(start * SUB, rg * SUB))
            blk = load(rg * SUB, (rg + 1) * SUB)
            head = blk[:, :LANES] | (tokens[rg] & self.zero)
            parts.append(head if blk.shape[1] == LANES else jnp.concatenate([head, blk[:, LANES:]], axis=1))
            start = rg + 1
        if start < n_rg:
            parts.append(load(start * SUB, n_rg * SUB))
        return _halves(parts[0] if len(parts) == 1 else jnp.concatenate(parts, axis=0))


def _kernel(
    x_hbm, wqkv_hbm, wo_hbm, w1_hbm, w2_hbm, b1_hbm, b2_hbm,
    out_hbm,
    x_v, wqkv_v, wo_v, w1_v, w2_v, b1_v, b2_v, zero_src, zero_v,
    wqkv_w, wo_f, wo_p, wo_w,
    xn_f, xn_w, h_cur, h_nxt, xn_tok, u_f, g_w,
    q_f, k_f, v_f, o_w, o_tok, y_f, out_v,
    sem_x, sem_w1, sem_misc, sem_out,
    *, S, D, F,
):
    DH = D // H
    NT = S // LANES
    NF = F // LANES
    HALO = W - 1
    D_RG = D // RG
    scale = DH ** -0.5
    dsplits = _lane_splits(D)
    sched = _Schedule()

    C1 = S // T1
    TPC = T1 // LANES

    def cp_x(c):
        sl = _ds(c * T1, T1)
        return pltpu.make_async_copy(x_hbm.at[:, sl], x_v.at[:, sl], sem_x.at[c])

    def cp_w1(c):
        sl = _ds(c * T1, T1)
        return pltpu.make_async_copy(w1_hbm.at[sl, :], w1_v.at[sl, :], sem_w1.at[c])

    cp_w1_head = pltpu.make_async_copy(
        w1_hbm.at[0:T1, 0:W1_HEAD], w1_v.at[0:T1, 0:W1_HEAD], sem_misc.at[6])
    cp_w1_rest = pltpu.make_async_copy(
        w1_hbm.at[0:T1, W1_HEAD:F], w1_v.at[0:T1, W1_HEAD:F], sem_w1.at[0])
    cp_b1 = pltpu.make_async_copy(b1_hbm, b1_v, sem_misc.at[0])
    cp_b2 = pltpu.make_async_copy(b2_hbm, b2_v, sem_misc.at[1])
    cp_wqkv = pltpu.make_async_copy(wqkv_hbm, wqkv_v, sem_misc.at[2])
    cp_wo = pltpu.make_async_copy(wo_hbm, wo_v, sem_misc.at[3])
    cp_w2 = pltpu.make_async_copy(w2_hbm, w2_v, sem_misc.at[4])
    cp_zero = pltpu.make_async_copy(zero_src, zero_v, sem_misc.at[5])
    starts_out = [sum(OUT_CHUNKS[:c]) for c in range(len(OUT_CHUNKS))]
    cp_out = [
        pltpu.make_async_copy(out_v.at[:, s0:s0 + n], out_hbm.at[:, s0:s0 + n], sem_out.at[c])
        for c, (s0, n) in enumerate(zip(starts_out, OUT_CHUNKS))
    ]

    cp_x(0).start()
    zero_src[...] = jnp.zeros((SUB, LANES), U32)
    cp_zero.start()
    cp_b1.start()
    cp_w1_head.start()
    cp_w1_rest.start()
    cp_x(1).start()

    def prefetch(c, carry):
        cp_w1(c).start()
        cp_x(c + 1).start()
        return carry

    lax.fori_loop(1, C1 - 1, prefetch, 0)
    cp_w1(C1 - 1).start()
    cp_wqkv.start()
    cp_wo.start()

    def norm_jobs(t, slot, h_dst):
        ls = _ds(t * LANES, LANES)
        hs = slice(slot * LANES, (slot + 1) * LANES)
        st = {}

        def mean1():
            st["m"] = _col_mean(x_v[:, ls].astype(F32))
            return [_bits(st["m"])]

        def var1():
            xc = x_v[:, ls].astype(F32) - st["m"]
            st["r"] = lax.rsqrt(_col_mean(xc * xc) + EPS)
            return [_bits(st["r"])]

        def apply1():
            xn = (x_v[:, ls].astype(F32) - st["m"]) * st["r"]
            xn_f[slot] = xn
            xn_w[slot] = _words(xn)
            st["m2"] = _col_mean(xn)
            return [_bits(st["m2"])]

        def transpose(i):
            def job():
                s0, w = dsplits[i]
                tw = pltpu.bitcast(_halves(xn_w[slot, s0 // 2:(s0 + w) // 2, :]).T, U32)
                dst = xn_tok.at[i, _ds(t * (4 * TOK_PITCH), 4 * TOK_PITCH, SUB), :]
                for q in range(4):
                    dst[q * TOK_PITCH:q * TOK_PITCH + NT, 0:w] = tw[q * NT:(q + 1) * NT]
                return [tw[-SUB:]] if w == LANES else []
            return job

        def var2():
            xc = xn_f[slot] - st["m2"]
            st["r2"] = lax.rsqrt(_col_mean(xc * xc) + EPS)
            return [_bits(st["r2"])]

        def apply2(a, b):
            def job():
                hw = _words((xn_f[slot, a * RG:b * RG, :] - st["m2"]) * st["r2"])
                h_dst[a * SUB:b * SUB, hs] = hw
                return [hw[i * SUB:(i + 1) * SUB] for i in range(b - a)]
            return job

        q = D_RG // 4
        return ([(4, mean1), (7, var1), (9, apply1)] + [(1, transpose(i)) for i in range(len(dsplits))]
                + [(6, var2)] + [(2, apply2(i * q, (i + 1) * q)) for i in range(4)])

    def wqkv_jobs():
        def tile(i, o0, ow):
            def job():
                s0, w = dsplits[i]
                tw = pltpu.bitcast(wqkv_v[s0:s0 + w, o0:o0 + ow].T, U32)
                wqkv_w[o0 // 2:(o0 + ow) // 2, s0:s0 + w] = tw
                return [tw[-SUB:]] if w == LANES else []
            return job
        return [(1, tile(i, o0, ow)) for o0, ow in _lane_splits(3 * D) for i in range(len(dsplits))]

    def wo_jobs():
        def widen(i):
            def job():
                s0, w = dsplits[i]
                v = wo_v[:, s0:s0 + w].astype(F32)
                wo_f[i, :, 0:w] = v
                return [_bits(v[-SUB:])] if w == LANES else []
            return job

        def regroup(d):
            def job():
                rows = [wo_f[i, pl.ds(d, H, stride=DH), :][:, 0:w] for i, (s0, w) in enumerate(dsplits)]
                pw = _words(jnp.concatenate(rows, axis=1))
                wo_p[d * SUB:(d + 1) * SUB, :] = pw
                return [pw[:, :LANES]]
            return job

        def turn(i, o0, ow):
            def job():
                s0, w = dsplits[i]
                tw = pltpu.bitcast(_halves(wo_p[s0 // 2:(s0 + w) // 2, o0:o0 + ow]).T, U32)
                wo_w[o0 // 2:(o0 + ow) // 2, s0:s0 + w] = tw
                return [tw[-SUB:]] if w == LANES else []
            return job

        return ([(2, widen(i)) for i in range(len(dsplits))] + [(1, regroup(d)) for d in range(DH)]
                + [(1, turn(i, o0, ow)) for i in range(len(dsplits)) for o0, ow in dsplits])

    N1 = 4 * LANES * LANES // T1
    U1 = F // N1

    def mix_units(c, lo, hi, jobs, first=False):
        sched.spread(jobs, [(i, rg) for i in range(lo, hi) for rg in range(D_RG)])
        for i in range(lo, hi):
            cols = slice(i * N1, (i + 1) * N1)
            lhs = sched.operand(i, lambda a, b: h_cur[a:b, :], D_RG)
            r = lax.dot_general(lhs, w1_v[_ds(c * T1, T1), cols], _NN, preferred_element_type=F32)
            u_f[:, cols] = r + (b1[:, cols] if first else u_f[:, cols])

    def next_norm_jobs(c):
        return [job for k in range(TPC) for job in norm_jobs((c + 1) * TPC + k, k, h_nxt)]

    cp_x(0).wait()
    for step in zip(*[norm_jobs(t, t, h_cur) for t in range(TPC)]):
        for _, job in step:
            job()
    cp_zero.wait()
    cp_b1.wait()
    cp_w1_head.wait()
    sched.zero = zero_v[...]
    b1 = b1_v[...].astype(F32).reshape(1, F)

    mix_units(0, 0, W1_HEAD // N1, [], first=True)
    cp_w1_rest.wait()
    cp_x(1).wait()
    mix_units(0, W1_HEAD // N1, U1, next_norm_jobs(0), first=True)
    h_cur[...] = h_nxt[...]

    def chunk(c, carry):
        cp_w1(c).wait()
        cp_x(c + 1).wait()

        sched.zero = zero_v[...]
        mix_units(c, 0, U1, next_norm_jobs(c))
        h_cur[...] = h_nxt[...]
        return carry

    lax.fori_loop(1, C1 - 1, chunk, 0)

    cp_w1(C1 - 1).wait()
    cp_wqkv.wait()
    cp_b2.start()
    cp_w2.start()
    sched.zero = zero_v[...]
    mix_units(C1 - 1, 0, U1, wqkv_jobs())

    order2 = list(range(NT - HALO, NT)) + list(range(NT - HALO))

    def gelu_jobs(f):
        def job(rg):
            def run():
                gw = _words(_gelu(u_f[rg * RG:(rg + 1) * RG, f * LANES:(f + 1) * LANES]))
                g_w[rg * SUB:(rg + 1) * SUB, f * LANES:(f + 1) * LANES] = gw
                return [gw]
            return run
        return [(3, job(rg)) for rg in range(D_RG)]

    GAP = SKEW[4]
    HALF = D // 2

    def skew(ref, t):
        return SKEW[0] if ref is q_f else SKEW[1] if ref is k_f else SKEW[2 + t % 2]

    def put_tile(ref, t, val):
        o = skew(ref, t)
        ref[t, o:o + HALF, :] = val[:HALF]
        ref[t, o + HALF + GAP:o + D + GAP, :] = val[HALF:]

    def head_rows(ref, t, d):
        o = skew(ref, t) + d
        return jnp.concatenate([ref[t, pl.ds(o, H // 2, stride=DH), :],
                                ref[t, pl.ds(o + HALF + GAP, H // 2, stride=DH), :]], axis=0)

    def halo_jobs(j):
        src, dst = j + HALO, j + HALO - NT

        def job(ref, a, b):
            def run():
                gap = GAP if a >= HALF else 0
                r = pltpu.roll(ref[src, skew(ref, src) + gap + a:skew(ref, src) + gap + b, :], DIL, 1)
                ref[dst, skew(ref, dst) + gap + a:skew(ref, dst) + gap + b, :] = r
                return [_bits(r[i:i + SUB]) for i in range(0, b - a, 4 * SUB)]
            return run
        q = D // 4
        return [(4, job(ref, a, a + q)) for ref in (k_f, v_f) for a in range(0, D, q)]

    n_qkv_rg = 3 * D // RG
    gelu_all = [job for f in range(NF) for job in gelu_jobs(f)]
    per = -(-len(gelu_all) // 15)
    wo_prep = wo_jobs()
    for i, j in enumerate(order2):
        jobs = gelu_all[i * per:(i + 1) * per] if i < 15 else []
        if i >= 1 and order2[i - 1] >= NT - HALO:
            halo = halo_jobs(order2[i - 1])
            jobs = jobs[:len(jobs) // 2] + halo + jobs[len(jobs) // 2:]
        if i >= 9:
            k = -(-len(wo_prep) // 7)
            jobs = jobs + wo_prep[(i - 9) * k:(i - 8) * k]
        sched.spread(jobs, [(("p2", i), rg) for rg in range(n_qkv_rg)])

    cp_wo.wait()
    for i, j in enumerate(order2):
        cols = [
            _halves(xn_tok[a, pl.ds(j, LANES // 2, stride=TOK_PITCH), :])[:, 0:w]
            for a, (s0, w) in enumerate(dsplits)
        ]
        rows = jnp.concatenate(cols, axis=1)
        lhs = sched.operand(("p2", i), lambda a, b: wqkv_w[a:b, :], n_qkv_rg)
        r = lax.dot_general(lhs, rows, _NT, preferred_element_type=F32)
        put_tile(q_f, j, r[0:D])
        put_tile(k_f, j + HALO, r[D:2 * D])
        put_tile(v_f, j + HALO, r[2 * D:3 * D])

    lane = lax.broadcasted_iota(jnp.int32, (H, LANES), 1)

    def attention_jobs(j):
        st = {}

        def logits(w):
            def job():
                acc = None
                for d in range(DH):
                    t = head_rows(q_f, j, d) * head_rows(k_f, j + HALO - w, d)
                    acc = t if acc is None else acc + t
                acc = acc * scale
                if w > j:
                    acc = jnp.where(lane < DIL, -1e9, acc)
                st[w] = acc
                return [_bits(acc[:SUB]), _bits(acc[SUB:])]
            return job

        def softmax():
            mx = st[0]
            for w in range(1, W):
                mx = jnp.maximum(mx, st[w])
            e = [jnp.exp(st[w] - mx) for w in range(W)]
            den = e[0]
            for w in range(1, W):
                den = den + e[w]
            inv = 1.0 / den
            st["p"] = [e[w] * inv for w in range(W)]
            return [_bits(p[a:a + SUB]) for p in st["p"] for a in (0, SUB)]

        def values(d):
            def job():
                acc = None
                for w in range(W):
                    t = st["p"][w] * head_rows(v_f, j + HALO - w, d)
                    acc = t if acc is None else acc + t
                ow = _words(acc)
                o_w[j, d * SUB:(d + 1) * SUB, :] = ow
                return [ow]
            return job

        def scatter(i):
            def job():
                s0, w = dsplits[i]
                tw = pltpu.bitcast(_halves(o_w[j, s0 // 2:(s0 + w) // 2, :]).T, U32)
                o_tok[i, j * ATT_PITCH:j * ATT_PITCH + LANES // 2, 0:w] = tw
                return [tw[-SUB:]] if w == LANES else []
            return job

        core = [(110, logits(w)) for w in range(W)] + [(130, softmax)]
        core += [(32, values(d)) for d in range(DH)]
        return core, [(20, scatter(i)) for i in range(len(dsplits))]

    kgroups = [(k0, min(4 * LANES, F - k0)) for k0 in range(0, F, 4 * LANES)]

    def slots3(ns):
        return [(("p3", n, g), rg) for n in ns for g, (k0, kw) in enumerate(kgroups)
                if kw == 4 * LANES for rg in range(D_RG)]

    att = [attention_jobs(j) for j in range(NT)]
    sched.spread([job for j in range(NT) for job in att[j][0]], slots3(range(ATT_TILES)))
    sched.spread([job for j in range(NT) for job in att[j][1]], slots3(range(ATT_TILES, NT)))

    cp_b2.wait()
    cp_w2.wait()
    b2 = b2_v[...].astype(F32).reshape(1, S)
    for n in range(NT):
        ls = slice(n * LANES, (n + 1) * LANES)
        for g, (k0, kw) in enumerate(kgroups):
            lhs = sched.operand(("p3", n, g), lambda a, b: g_w[a:b, k0:k0 + kw], D_RG)
            r = lax.dot_general(lhs, w2_v[k0:k0 + kw, ls], _NN, preferred_element_type=F32)
            if g == 0:
                y_f[:, ls] = r + b2[:, ls]
            else:
                y_f[:, ls] += r

    ends_out = {s0 + n: c for c, (s0, n) in enumerate(zip(starts_out, OUT_CHUNKS))}
    for n in range(NT):
        ls = slice(n * LANES, (n + 1) * LANES)
        cols = [
            jnp.concatenate(
                [_halves(o_tok[a, pl.ds(4 * n + q, NT, stride=ATT_PITCH), :]) for q in range(4)], axis=0
            )[:, 0:w]
            for a, (s0, w) in enumerate(dsplits)
        ]
        o = jnp.concatenate(cols, axis=1)
        lhs = sched.operand(("p4", n), lambda a, b: wo_w[a:b, :], D_RG)
        a = lax.dot_general(lhs, o, _NT, preferred_element_type=F32)
        out_v[:, ls] = (x_v[:, ls].astype(F32) + a + y_f[:, ls]).astype(BF16)
        if (n + 1) * LANES in ends_out:
            cp_out[ends_out[(n + 1) * LANES]].start()
    assert not sched.plan, list(sched.plan)
    for cp in cp_out:
        cp.wait()


@jax.jit
def pallas_parallel_sum__sliding_local_dilated__mixer_token_mlp__prompt_kernel(
    A_x: jax.Array,
    A_wqkv: jax.Array,
    A_wo: jax.Array,
    B_x: jax.Array,
    B_w1: jax.Array,
    B_b1: jax.Array,
    B_w2: jax.Array,
    B_b2: jax.Array,
):
    del B_x
    Bsz, S, D = A_x.shape
    F = B_w1.shape[1]
    assert Bsz == 1 and S == 16 * LANES and D % H == 0 and D % (4 * RG) == 0 and F % LANES == 0
    assert S % T1 == 0 and S // T1 >= 5 and sum(OUT_CHUNKS) == S
    nct = -(-D // LANES)
    NT = S // LANES
    HALO = W - 1

    x_t = A_x.reshape(S, D).T

    def kern(*refs):
        _kernel(*refs, S=S, D=D, F=F)

    hbm = pl.BlockSpec(memory_space=pl.ANY)
    scratch = [
        pltpu.VMEM((D, S), BF16),
        pltpu.VMEM((D, 3 * D), BF16),
        pltpu.VMEM((D, D), BF16),
        pltpu.VMEM((S, F), BF16),
        pltpu.VMEM((F, S), BF16),
        pltpu.VMEM((F,), BF16),
        pltpu.VMEM((S,), BF16),
        pltpu.VMEM((SUB, LANES), U32),
        pltpu.VMEM((SUB, LANES), U32),
        pltpu.VMEM((3 * D // 2, D), U32),
        pltpu.VMEM((nct, D, LANES), F32),
        pltpu.VMEM((D // 2, D), U32),
        pltpu.VMEM((D // 2, D), U32),
        pltpu.VMEM((T1 // LANES, D, LANES), F32),
        pltpu.VMEM((T1 // LANES, D // 2, LANES), U32),
        pltpu.VMEM((D // 2, T1), U32),
        pltpu.VMEM((D // 2, T1), U32),
        pltpu.VMEM((nct, (S // 32) * TOK_PITCH, LANES), U32),
        pltpu.VMEM((D, F), F32),
        pltpu.VMEM((D // 2, F), U32),
        pltpu.VMEM((NT, D + SUB, LANES), F32),
        pltpu.VMEM((NT + HALO, D + SUB, LANES), F32),
        pltpu.VMEM((NT + HALO, D + SUB, LANES), F32),
        pltpu.VMEM((NT, D // 2, LANES), U32),
        pltpu.VMEM((nct, NT * ATT_PITCH, LANES), U32),
        pltpu.VMEM((D, S), F32),
        pltpu.VMEM((D, S), BF16),
        pltpu.SemaphoreType.DMA((S // T1,)),
        pltpu.SemaphoreType.DMA((S // T1,)),
        pltpu.SemaphoreType.DMA((7,)),
        pltpu.SemaphoreType.DMA((len(OUT_CHUNKS),)),
    ]
    out_t = pl.pallas_call(
        kern,
        out_shape=jax.ShapeDtypeStruct((D, S), BF16),
        in_specs=[hbm] * 7,
        out_specs=hbm,
        scratch_shapes=scratch,
        compiler_params=pltpu.CompilerParams(vmem_limit_bytes=100 * 1024 * 1024),
    )(x_t, A_wqkv, A_wo, B_w1, B_w2, B_b1, B_b2)
    return out_t.T.reshape(1, S, D)
```

```python
import math

import jax
import jax.numpy as jnp
from jax import lax
from jax.experimental import pallas as pl
from jax.experimental.pallas import tpu as pltpu

F32 = jnp.float32
BF16 = jnp.bfloat16
U32 = jnp.uint32

H = 16
W = 8
DIL = 2
LANES = 128
SUB = 8
RG = 16
EPS = 1e-5

T1 = 256
OUT_CHUNKS = (256, 256, 256, 256, 256, 256, 256, 128, 128)
SKIP3 = 8
LOOPED = 5
PAIR = 2
SKEW = (0, 1, 0, 1, 2)
W1_HEAD = 768
ATT_TILES = 15
TOK_PITCH = 18
ATT_PITCH = 66

_NN = (((1,), (0,)), ((), ()))
_NT = (((1,), (1,)), ((), ()))
_GELU_C = math.sqrt(2.0 / math.pi)


def _ds(start, size, align=None):
    if isinstance(start, int):
        return pl.ds(start, size)
    return pl.ds(pl.multiple_of(start, align or size), size)


def _lane_splits(n):
    return [(s, min(LANES, n - s)) for s in range(0, n, LANES)]


def _words(v):
    return pltpu.bitcast(v.astype(BF16), U32)


def _halves(w):
    return pltpu.bitcast(w, BF16)


def _bits(v):
    return pltpu.bitcast(jnp.broadcast_to(v, (SUB, LANES)), U32)


def _gelu(u):
    inner = _GELU_C * (u + 0.044715 * (u * u * u))
    return 0.5 * u * (1.0 + jnp.tanh(inner))


def _col_mean(v):
    acc = v[0:SUB]
    for i in range(1, v.shape[0] // SUB):
        acc = acc + v[i * SUB:(i + 1) * SUB]
    return jnp.sum(acc, axis=0, keepdims=True) / v.shape[0]


class _Schedule:
    def __init__(self):
        self.zero = None
        self.plan = {}

    def spread(self, jobs, slots):
        total = sum(c for c, _ in jobs)
        done = 0
        for cost, fn in jobs:
            done += cost
            unit, rg = slots[min(len(slots) - 1, (done * len(slots) - 1) // total)]
            self.plan.setdefault(unit, []).append((rg, fn))

    def operand(self, unit, load, n_rg):
        tokens = {}
        for rg, fn in self.plan.pop(unit, []):
            for t in fn() or []:
                tokens[rg] = t if rg not in tokens else tokens[rg] | t
        parts, start = [], 0
        for rg in sorted(tokens):
            if rg > start:
                parts.append(load(start * SUB, rg * SUB))
            blk = load(rg * SUB, (rg + 1) * SUB)
            head = blk[:, :LANES] | (tokens[rg] & self.zero)
            parts.append(head if blk.shape[1] == LANES else jnp.concatenate([head, blk[:, LANES:]], axis=1))
            start = rg + 1
        if start < n_rg:
            parts.append(load(start * SUB, n_rg * SUB))
        return _halves(parts[0] if len(parts) == 1 else jnp.concatenate(parts, axis=0))


def _kernel(
    x_hbm, wqkv_hbm, wo_hbm, w1_hbm, w2_hbm, b1_hbm, b2_hbm,
    out_hbm,
    x_v, wqkv_v, wo_v, w1_v, w2_v, b1_v, b2_v, zero_src, zero_v,
    wqkv_w, wo_f, wo_p, wo_w,
    xn_f, xn_w, h_cur, h_nxt, xn_tok, u_f, g_w,
    q_f, k_f, v_f, o_w, o_tok, y_f, out_v,
    sem_x, sem_w1, sem_misc, sem_out,
    *, S, D, F,
):
    DH = D // H
    NT = S // LANES
    NF = F // LANES
    HALO = W - 1
    D_RG = D // RG
    scale = DH ** -0.5
    dsplits = _lane_splits(D)
    sched = _Schedule()

    C1 = S // T1
    TPC = T1 // LANES

    def cp_x(c):
        sl = _ds(c * T1, T1)
        return pltpu.make_async_copy(x_hbm.at[:, sl], x_v.at[:, sl], sem_x.at[c])

    def cp_w1(c):
        sl = _ds(c * T1, T1)
        return pltpu.make_async_copy(w1_hbm.at[sl, :], w1_v.at[sl, :], sem_w1.at[c])

    cp_w1_head = pltpu.make_async_copy(
        w1_hbm.at[0:T1, 0:W1_HEAD], w1_v.at[0:T1, 0:W1_HEAD], sem_misc.at[6])
    cp_w1_rest = pltpu.make_async_copy(
        w1_hbm.at[0:T1, W1_HEAD:F], w1_v.at[0:T1, W1_HEAD:F], sem_w1.at[0])
    cp_b1 = pltpu.make_async_copy(b1_hbm, b1_v, sem_misc.at[0])
    cp_b2 = pltpu.make_async_copy(b2_hbm, b2_v, sem_misc.at[1])
    cp_wqkv = pltpu.make_async_copy(wqkv_hbm, wqkv_v, sem_misc.at[2])
    cp_wo = pltpu.make_async_copy(wo_hbm, wo_v, sem_misc.at[3])
    cp_w2 = pltpu.make_async_copy(w2_hbm, w2_v, sem_misc.at[4])
    cp_zero = pltpu.make_async_copy(zero_src, zero_v, sem_misc.at[5])
    starts_out = [sum(OUT_CHUNKS[:c]) for c in range(len(OUT_CHUNKS))]
    cp_out = [
        pltpu.make_async_copy(out_v.at[:, s0:s0 + n], out_hbm.at[:, s0:s0 + n], sem_out.at[c])
        for c, (s0, n) in enumerate(zip(starts_out, OUT_CHUNKS))
    ]

    cp_x(0).start()
    zero_src[...] = jnp.zeros((SUB, LANES), U32)
    cp_zero.start()
    cp_b1.start()
    cp_w1_head.start()
    cp_w1_rest.start()
    cp_x(1).start()

    def prefetch(c, carry):
        cp_w1(c).start()
        cp_x(c + 1).start()
        return carry

    lax.fori_loop(1, C1 - 1, prefetch, 0)
    cp_w1(C1 - 1).start()
    cp_wqkv.start()
    cp_wo.start()

    def norm_jobs(t, slot, h_dst):
        ls = _ds(t * LANES, LANES)
        hs = slice(slot * LANES, (slot + 1) * LANES)
        st = {}

        def mean1():
            st["m"] = _col_mean(x_v[:, ls].astype(F32))
            return [_bits(st["m"])]

        def var1():
            xc = x_v[:, ls].astype(F32) - st["m"]
            st["r"] = lax.rsqrt(_col_mean(xc * xc) + EPS)
            return [_bits(st["r"])]

        def apply1():
            xn = (x_v[:, ls].astype(F32) - st["m"]) * st["r"]
            xn_f[slot] = xn
            xn_w[slot] = _words(xn)
            st["m2"] = _col_mean(xn)
            return [_bits(st["m2"])]

        def transpose(i):
            def job():
                s0, w = dsplits[i]
                tw = pltpu.bitcast(_halves(xn_w[slot, s0 // 2:(s0 + w) // 2, :]).T, U32)
                dst = xn_tok.at[i, _ds(t * (4 * TOK_PITCH), 4 * TOK_PITCH, SUB), :]
                for q in range(4):
                    dst[q * TOK_PITCH:q * TOK_PITCH + NT, 0:w] = tw[q * NT:(q + 1) * NT]
                return [tw[-SUB:]] if w == LANES else []
            return job

        def var2():
            xc = xn_f[slot] - st["m2"]
            st["r2"] = lax.rsqrt(_col_mean(xc * xc) + EPS)
            return [_bits(st["r2"])]

        def apply2(a, b):
            def job():
                hw = _words((xn_f[slot, a * RG:b * RG, :] - st["m2"]) * st["r2"])
                h_dst[a * SUB:b * SUB, hs] = hw
                return [hw[i * SUB:(i + 1) * SUB] for i in range(b - a)]
            return job

        q = D_RG // 4
        return ([(4, mean1), (7, var1), (9, apply1)] + [(1, transpose(i)) for i in range(len(dsplits))]
                + [(6, var2)] + [(2, apply2(i * q, (i + 1) * q)) for i in range(4)])

    def wqkv_jobs():
        def tile(i, o0, ow):
            def job():
                s0, w = dsplits[i]
                tw = pltpu.bitcast(wqkv_v[s0:s0 + w, o0:o0 + ow].T, U32)
                wqkv_w[o0 // 2:(o0 + ow) // 2, s0:s0 + w] = tw
                return [tw[-SUB:]] if w == LANES else []
            return job
        return [(1, tile(i, o0, ow)) for o0, ow in _lane_splits(3 * D) for i in range(len(dsplits))]

    def wo_jobs():
        def widen(i):
            def job():
                s0, w = dsplits[i]
                v = wo_v[:, s0:s0 + w].astype(F32)
                wo_f[i, :, 0:w] = v
                return [_bits(v[-SUB:])] if w == LANES else []
            return job

        def regroup(d):
            def job():
                rows = [wo_f[i, pl.ds(d, H, stride=DH), :][:, 0:w] for i, (s0, w) in enumerate(dsplits)]
                pw = _words(jnp.concatenate(rows, axis=1))
                wo_p[d * SUB:(d + 1) * SUB, :] = pw
                return [pw[:, :LANES]]
            return job

        def turn(i, o0, ow):
            def job():
                s0, w = dsplits[i]
                tw = pltpu.bitcast(_halves(wo_p[s0 // 2:(s0 + w) // 2, o0:o0 + ow]).T, U32)
                wo_w[o0 // 2:(o0 + ow) // 2, s0:s0 + w] = tw
                return [tw[-SUB:]] if w == LANES else []
            return job

        return ([(2, widen(i)) for i in range(len(dsplits))] + [(1, regroup(d)) for d in range(DH)]
                + [(1, turn(i, o0, ow)) for i in range(len(dsplits)) for o0, ow in dsplits])

    N1 = 4 * LANES * LANES // T1
    U1 = F // N1

    def mix_units(c, lo, hi, jobs, first=False, h_cur=h_cur):
        sched.spread(jobs, [(i, rg) for i in range(lo, hi) for rg in range(D_RG)])
        for i in range(lo, hi):
            cols = slice(i * N1, (i + 1) * N1)
            lhs = sched.operand(i, lambda a, b: h_cur[a:b, :], D_RG)
            r = lax.dot_general(lhs, w1_v[_ds(c * T1, T1), cols], _NN, preferred_element_type=F32)
            u_f[:, cols] = r + (b1[:, cols] if first else u_f[:, cols])

    def next_norm_jobs(c, h_nxt=h_nxt):
        return [job for k in range(TPC) for job in norm_jobs((c + 1) * TPC + k, k, h_nxt)]

    cp_x(0).wait()
    for step in zip(*[norm_jobs(t, t, h_cur) for t in range(TPC)]):
        for _, job in step:
            job()
    cp_zero.wait()
    cp_b1.wait()
    cp_w1_head.wait()
    sched.zero = zero_v[...]
    b1 = b1_v[...].astype(F32).reshape(1, F)

    mix_units(0, 0, W1_HEAD // N1, [], first=True)
    cp_w1_rest.wait()
    cp_x(1).wait()
    mix_units(0, W1_HEAD // N1, U1, next_norm_jobs(0), first=True)
    h_cur[...] = h_nxt[...]

    def chunk(c, carry):
        cp_w1(c).wait()
        cp_x(c + 1).wait()

        sched.zero = zero_v[...]
        mix_units(c, 0, U1, next_norm_jobs(c))
        h_cur[...] = h_nxt[...]
        return carry

    lax.fori_loop(1, LOOPED + 1, chunk, 0)

    bufs = [h_cur, h_nxt]
    for c0 in range(LOOPED + 1, C1, PAIR):
        block = range(c0, min(C1, c0 + PAIR))
        for c in block:
            cp_w1(c).wait()
            if c + 1 < C1:
                cp_x(c + 1).wait()
            else:
                cp_wqkv.wait()
                cp_wo.wait()
                cp_b2.start()
                cp_w2.start()
        sched.zero = zero_v[...]
        for c in block:
            jobs = next_norm_jobs(c, bufs[1]) if c + 1 < C1 else wqkv_jobs()
            mix_units(c, 0, U1, jobs, h_cur=bufs[0])
            bufs.reverse()

    order2 = list(range(NT - HALO, NT)) + list(range(NT - HALO))

    def gelu_jobs(f):
        def job(rg):
            def run():
                gw = _words(_gelu(u_f[rg * RG:(rg + 1) * RG, f * LANES:(f + 1) * LANES]))
                g_w[rg * SUB:(rg + 1) * SUB, f * LANES:(f + 1) * LANES] = gw
                return [gw]
            return run
        return [(3, job(rg)) for rg in range(D_RG)]

    GAP = SKEW[4]
    HALF = D // 2

    def skew(ref, t):
        return SKEW[0] if ref is q_f else SKEW[1] if ref is k_f else SKEW[2 + t % 2]

    def put_tile(ref, t, val):
        o = skew(ref, t)
        ref[t, o:o + HALF, :] = val[:HALF]
        ref[t, o + HALF + GAP:o + D + GAP, :] = val[HALF:]

    def head_rows(ref, t, d):
        o = skew(ref, t) + d
        return jnp.concatenate([ref[t, pl.ds(o, H // 2, stride=DH), :],
                                ref[t, pl.ds(o + HALF + GAP, H // 2, stride=DH), :]], axis=0)

    def halo_jobs(j):
        src, dst = j + HALO, j + HALO - NT

        def job(ref, a, b):
            def run():
                gap = GAP if a >= HALF else 0
                r = pltpu.roll(ref[src, skew(ref, src) + gap + a:skew(ref, src) + gap + b, :], DIL, 1)
                ref[dst, skew(ref, dst) + gap + a:skew(ref, dst) + gap + b, :] = r
                return [_bits(r[i:i + SUB]) for i in range(0, b - a, 4 * SUB)]
            return run
        q = D // 4
        return [(4, job(ref, a, a + q)) for ref in (k_f, v_f) for a in range(0, D, q)]

    n_qkv_rg = 3 * D // RG
    gelu_all = [job for f in range(NF) for job in gelu_jobs(f)]
    per = -(-len(gelu_all) // 15)
    wo_prep = wo_jobs()
    for i, j in enumerate(order2):
        jobs = gelu_all[i * per:(i + 1) * per] if i < 15 else []
        if i >= 1 and order2[i - 1] >= NT - HALO:
            halo = halo_jobs(order2[i - 1])
            jobs = jobs[:len(jobs) // 2] + halo + jobs[len(jobs) // 2:]
        if i >= 9:
            k = -(-len(wo_prep) // 7)
            jobs = jobs + wo_prep[(i - 9) * k:(i - 8) * k]
        sched.spread(jobs, [(("p2", i), rg) for rg in range(n_qkv_rg)])

    for i, j in enumerate(order2):
        cols = [
            _halves(xn_tok[a, pl.ds(j, LANES // 2, stride=TOK_PITCH), :])[:, 0:w]
            for a, (s0, w) in enumerate(dsplits)
        ]
        rows = jnp.concatenate(cols, axis=1)
        lhs = sched.operand(("p2", i), lambda a, b: wqkv_w[a:b, :], n_qkv_rg)
        r = lax.dot_general(lhs, rows, _NT, preferred_element_type=F32)
        put_tile(q_f, j, r[0:D])
        put_tile(k_f, j + HALO, r[D:2 * D])
        put_tile(v_f, j + HALO, r[2 * D:3 * D])

    lane = lax.broadcasted_iota(jnp.int32, (H, LANES), 1)

    def attention_jobs(j):
        st = {}

        def logits(w):
            def job():
                acc = None
                for d in range(DH):
                    t = head_rows(q_f, j, d) * head_rows(k_f, j + HALO - w, d)
                    acc = t if acc is None else acc + t
                acc = acc * scale
                if w > j:
                    acc = jnp.where(lane < DIL, -1e9, acc)
                st[w] = acc
                return [_bits(acc[:SUB]), _bits(acc[SUB:])]
            return job

        def softmax():
            mx = st[0]
            for w in range(1, W):
                mx = jnp.maximum(mx, st[w])
            e = [jnp.exp(st[w] - mx) for w in range(W)]
            den = e[0]
            for w in range(1, W):
                den = den + e[w]
            inv = 1.0 / den
            st["p"] = [e[w] * inv for w in range(W)]
            return [_bits(p[a:a + SUB]) for p in st["p"] for a in (0, SUB)]

        def values(d):
            def job():
                acc = None
                for w in range(W):
                    t = st["p"][w] * head_rows(v_f, j + HALO - w, d)
                    acc = t if acc is None else acc + t
                ow = _words(acc)
                o_w[j, d * SUB:(d + 1) * SUB, :] = ow
                return [ow]
            return job

        def scatter(i):
            def job():
                s0, w = dsplits[i]
                tw = pltpu.bitcast(_halves(o_w[j, s0 // 2:(s0 + w) // 2, :]).T, U32)
                o_tok[i, j * ATT_PITCH:j * ATT_PITCH + LANES // 2, 0:w] = tw
                return [tw[-SUB:]] if w == LANES else []
            return job

        core = [(110, logits(w)) for w in range(W)] + [(130, softmax)]
        core += [(32, values(d)) for d in range(DH)]
        return core, [(20, scatter(i)) for i in range(len(dsplits))]

    KG = 4 * LANES
    n_full, k_tail = F // KG, F % KG
    wide = KG // k_tail if k_tail else 1
    units3 = []
    for n0 in range(0, NT, wide):
        units3 += [(n, 1, g * KG, KG) for n in range(n0, n0 + wide) for g in range(n_full)]
        if k_tail:
            units3.append((n0, wide, n_full * KG, k_tail))
    n_att = ATT_TILES * len(units3) // NT

    def slots3(lo, hi):
        return [(("p3", u), rg) for u in range(lo, hi) for rg in range(D_RG)]

    att = [attention_jobs(j) for j in range(NT)]
    sched.spread([job for j in range(NT) for job in att[j][0]], slots3(0, n_att)[SKIP3:])
    sched.spread([job for j in range(NT) for job in att[j][1]], slots3(n_att, len(units3)))

    cp_b2.wait()
    cp_w2.wait()
    b2 = b2_v[...].astype(F32).reshape(1, S)
    for u, (n, nn, k0, kw) in enumerate(units3):
        ls = slice(n * LANES, (n + nn) * LANES)
        lhs = sched.operand(("p3", u), lambda a, b: g_w[a:b, k0:k0 + kw], D_RG)
        r = lax.dot_general(lhs, w2_v[k0:k0 + kw, ls], _NN, preferred_element_type=F32)
        if k0 == 0:
            y_f[:, ls] = r + b2[:, ls]
        else:
            y_f[:, ls] += r

    ends_out = {s0 + n: c for c, (s0, n) in enumerate(zip(starts_out, OUT_CHUNKS))}
    for n in range(NT):
        ls = slice(n * LANES, (n + 1) * LANES)
        cols = [
            jnp.concatenate(
                [_halves(o_tok[a, pl.ds(4 * n + q, NT, stride=ATT_PITCH), :]) for q in range(4)], axis=0
            )[:, 0:w]
            for a, (s0, w) in enumerate(dsplits)
        ]
        o = jnp.concatenate(cols, axis=1)
        lhs = sched.operand(("p4", n), lambda a, b: wo_w[a:b, :], D_RG)
        a = lax.dot_general(lhs, o, _NT, preferred_element_type=F32)
        out_v[:, ls] = (x_v[:, ls].astype(F32) + a + y_f[:, ls]).astype(BF16)
        if (n + 1) * LANES in ends_out:
            cp_out[ends_out[(n + 1) * LANES]].start()
    assert not sched.plan, list(sched.plan)
    for cp in cp_out:
        cp.wait()


@jax.jit
def pallas_parallel_sum__sliding_local_dilated__mixer_token_mlp__prompt_kernel(
    A_x: jax.Array,
    A_wqkv: jax.Array,
    A_wo: jax.Array,
    B_x: jax.Array,
    B_w1: jax.Array,
    B_b1: jax.Array,
    B_w2: jax.Array,
    B_b2: jax.Array,
):
    del B_x
    Bsz, S, D = A_x.shape
    F = B_w1.shape[1]
    assert Bsz == 1 and S == 16 * LANES and D % H == 0 and D % (4 * RG) == 0 and F % LANES == 0
    assert (F % (4 * LANES)) in (0, LANES, 2 * LANES)
    assert S % T1 == 0 and S // T1 >= 5 and sum(OUT_CHUNKS) == S
    nct = -(-D // LANES)
    NT = S // LANES
    HALO = W - 1

    x_t = A_x.reshape(S, D).T

    def kern(*refs):
        _kernel(*refs, S=S, D=D, F=F)

    hbm = pl.BlockSpec(memory_space=pl.ANY)
    scratch = [
        pltpu.VMEM((D, S), BF16),
        pltpu.VMEM((D, 3 * D), BF16),
        pltpu.VMEM((D, D), BF16),
        pltpu.VMEM((S, F), BF16),
        pltpu.VMEM((F, S), BF16),
        pltpu.VMEM((F,), BF16),
        pltpu.VMEM((S,), BF16),
        pltpu.VMEM((SUB, LANES), U32),
        pltpu.VMEM((SUB, LANES), U32),
        pltpu.VMEM((3 * D // 2, D), U32),
        pltpu.VMEM((nct, D, LANES), F32),
        pltpu.VMEM((D // 2, D), U32),
        pltpu.VMEM((D // 2, D), U32),
        pltpu.VMEM((T1 // LANES, D, LANES), F32),
        pltpu.VMEM((T1 // LANES, D // 2, LANES), U32),
        pltpu.VMEM((D // 2, T1), U32),
        pltpu.VMEM((D // 2, T1), U32),
        pltpu.VMEM((nct, (S // 32) * TOK_PITCH, LANES), U32),
        pltpu.VMEM((D, F), F32),
        pltpu.VMEM((D // 2, F), U32),
        pltpu.VMEM((NT, D + SUB, LANES), F32),
        pltpu.VMEM((NT + HALO, D + SUB, LANES), F32),
        pltpu.VMEM((NT + HALO, D + SUB, LANES), F32),
        pltpu.VMEM((NT, D // 2, LANES), U32),
        pltpu.VMEM((nct, NT * ATT_PITCH, LANES), U32),
        pltpu.VMEM((D, S), F32),
        pltpu.VMEM((D, S), BF16),
        pltpu.SemaphoreType.DMA((S // T1,)),
        pltpu.SemaphoreType.DMA((S // T1,)),
        pltpu.SemaphoreType.DMA((7,)),
        pltpu.SemaphoreType.DMA((len(OUT_CHUNKS),)),
    ]
    out_t = pl.pallas_call(
        kern,
        out_shape=jax.ShapeDtypeStruct((D, S), BF16),
        in_specs=[hbm] * 7,
        out_specs=hbm,
        scratch_shapes=scratch,
        compiler_params=pltpu.CompilerParams(vmem_limit_bytes=100 * 1024 * 1024),
    )(x_t, A_wqkv, A_wo, B_w1, B_w2, B_b1, B_b2)
    return out_t.T.reshape(1, S, D)
```

```python
import math

import jax
import jax.numpy as jnp
from jax import lax
from jax.experimental import pallas as pl
from jax.experimental.pallas import tpu as pltpu

F32 = jnp.float32
BF16 = jnp.bfloat16
U32 = jnp.uint32

H = 16
W = 8
DIL = 2
LANES = 128
SUB = 8
RG = 16
EPS = 1e-5

T1 = 256
OUT_CHUNKS = (512, 512, 512, 256, 128, 128)
SKIP3 = 8
LOOPED = 5
PAIR = 2
SKEW = (0, 1, 0, 1, 2)
W1_HEAD = 768
ATT_TILES = 15
TOK_PITCH = 18
ATT_PITCH = 66

_NN = (((1,), (0,)), ((), ()))
_NT = (((1,), (1,)), ((), ()))
_GELU_C = math.sqrt(2.0 / math.pi)


def _ds(start, size, align=None):
    if isinstance(start, int):
        return pl.ds(start, size)
    return pl.ds(pl.multiple_of(start, align or size), size)


def _lane_splits(n):
    return [(s, min(LANES, n - s)) for s in range(0, n, LANES)]


def _words(v):
    return pltpu.bitcast(v.astype(BF16), U32)


def _halves(w):
    return pltpu.bitcast(w, BF16)


def _bits(v):
    return pltpu.bitcast(jnp.broadcast_to(v, (SUB, LANES)), U32)


def _gelu(u):
    inner = _GELU_C * (u + 0.044715 * (u * u * u))
    return 0.5 * u * (1.0 + jnp.tanh(inner))


def _col_mean(v):
    acc = v[0:SUB]
    for i in range(1, v.shape[0] // SUB):
        acc = acc + v[i * SUB:(i + 1) * SUB]
    return jnp.sum(acc, axis=0, keepdims=True) / v.shape[0]


class _Schedule:
    def __init__(self):
        self.zero = None
        self.plan = {}

    def spread(self, jobs, slots):
        total = sum(c for c, _ in jobs)
        done = 0
        for cost, fn in jobs:
            done += cost
            unit, rg = slots[min(len(slots) - 1, (done * len(slots) - 1) // total)]
            self.plan.setdefault(unit, []).append((rg, fn))

    def operand(self, unit, load, n_rg):
        tokens = {}
        for rg, fn in self.plan.pop(unit, []):
            for t in fn() or []:
                tokens[rg] = t if rg not in tokens else tokens[rg] | t
        parts, start = [], 0
        for rg in sorted(tokens):
            if rg > start:
                parts.append(load(start * SUB, rg * SUB))
            blk = load(rg * SUB, (rg + 1) * SUB)
            head = blk[:, :LANES] | (tokens[rg] & self.zero)
            parts.append(head if blk.shape[1] == LANES else jnp.concatenate([head, blk[:, LANES:]], axis=1))
            start = rg + 1
        if start < n_rg:
            parts.append(load(start * SUB, n_rg * SUB))
        return _halves(parts[0] if len(parts) == 1 else jnp.concatenate(parts, axis=0))


def _kernel(
    x_hbm, wqkv_hbm, wo_hbm, w1_hbm, w2_hbm, b1_hbm, b2_hbm,
    out_hbm,
    x_v, wqkv_v, wo_v, w1_v, w2_v, b1_v, b2_v, zero_src, zero_v,
    wqkv_w, wo_f, wo_p, wo_w,
    xn_f, xn_w, h_cur, h_nxt, xn_tok, u_f, g_w,
    q_f, k_f, v_f, o_w, o_tok, y_f, out_v,
    sem_x, sem_w1, sem_misc, sem_out,
    *, S, D, F,
):
    DH = D // H
    NT = S // LANES
    NF = F // LANES
    HALO = W - 1
    D_RG = D // RG
    scale = DH ** -0.5
    dsplits = _lane_splits(D)
    sched = _Schedule()

    C1 = S // T1
    TPC = T1 // LANES

    def cp_x(c):
        sl = _ds(c * T1, T1)
        return pltpu.make_async_copy(x_hbm.at[:, sl], x_v.at[:, sl], sem_x.at[c])

    def cp_w1(c):
        sl = _ds(c * T1, T1)
        return pltpu.make_async_copy(w1_hbm.at[sl, :], w1_v.at[sl, :], sem_w1.at[c])

    cp_w1_head = pltpu.make_async_copy(
        w1_hbm.at[0:T1, 0:W1_HEAD], w1_v.at[0:T1, 0:W1_HEAD], sem_misc.at[6])
    cp_w1_rest = pltpu.make_async_copy(
        w1_hbm.at[0:T1, W1_HEAD:F], w1_v.at[0:T1, W1_HEAD:F], sem_w1.at[0])
    cp_b1 = pltpu.make_async_copy(b1_hbm, b1_v, sem_misc.at[0])
    cp_b2 = pltpu.make_async_copy(b2_hbm, b2_v, sem_misc.at[1])
    cp_wqkv = pltpu.make_async_copy(wqkv_hbm, wqkv_v, sem_misc.at[2])
    cp_wo = pltpu.make_async_copy(wo_hbm, wo_v, sem_misc.at[3])
    cp_w2 = pltpu.make_async_copy(w2_hbm, w2_v, sem_misc.at[4])
    cp_zero = pltpu.make_async_copy(zero_src, zero_v, sem_misc.at[5])
    starts_out = [sum(OUT_CHUNKS[:c]) for c in range(len(OUT_CHUNKS))]
    cp_out = [
        pltpu.make_async_copy(out_v.at[:, s0:s0 + n], out_hbm.at[:, s0:s0 + n], sem_out.at[c])
        for c, (s0, n) in enumerate(zip(starts_out, OUT_CHUNKS))
    ]

    cp_x(0).start()
    zero_src[...] = jnp.zeros((SUB, LANES), U32)
    cp_zero.start()
    cp_b1.start()
    cp_w1_head.start()
    cp_w1_rest.start()
    cp_x(1).start()

    def prefetch(c, carry):
        cp_w1(c).start()
        cp_x(c + 1).start()
        return carry

    lax.fori_loop(1, C1 - 1, prefetch, 0)
    cp_w1(C1 - 1).start()
    cp_wqkv.start()
    cp_wo.start()

    def norm_jobs(t, slot, h_dst):
        ls = _ds(t * LANES, LANES)
        hs = slice(slot * LANES, (slot + 1) * LANES)
        st = {}

        def mean1():
            st["m"] = _col_mean(x_v[:, ls].astype(F32))
            return [_bits(st["m"])]

        def var1():
            xc = x_v[:, ls].astype(F32) - st["m"]
            st["r"] = lax.rsqrt(_col_mean(xc * xc) + EPS)
            return [_bits(st["r"])]

        def apply1():
            xn = (x_v[:, ls].astype(F32) - st["m"]) * st["r"]
            xn_f[slot] = xn
            xn_w[slot] = _words(xn)
            st["m2"] = _col_mean(xn)
            return [_bits(st["m2"])]

        def transpose(i):
            def job():
                s0, w = dsplits[i]
                tw = pltpu.bitcast(_halves(xn_w[slot, s0 // 2:(s0 + w) // 2, :]).T, U32)
                dst = xn_tok.at[i, _ds(t * (4 * TOK_PITCH), 4 * TOK_PITCH, SUB), :]
                for q in range(4):
                    dst[q * TOK_PITCH:q * TOK_PITCH + NT, 0:w] = tw[q * NT:(q + 1) * NT]
                return [tw[-SUB:]] if w == LANES else []
            return job

        def var2():
            xc = xn_f[slot] - st["m2"]
            st["r2"] = lax.rsqrt(_col_mean(xc * xc) + EPS)
            return [_bits(st["r2"])]

        def apply2(a, b):
            def job():
                hw = _words((xn_f[slot, a * RG:b * RG, :] - st["m2"]) * st["r2"])
                h_dst[a * SUB:b * SUB, hs] = hw
                return [hw[i * SUB:(i + 1) * SUB] for i in range(b - a)]
            return job

        q = D_RG // 4
        return ([(4, mean1), (7, var1), (9, apply1)] + [(1, transpose(i)) for i in range(len(dsplits))]
                + [(6, var2)] + [(2, apply2(i * q, (i + 1) * q)) for i in range(4)])

    def wqkv_jobs():
        def tile(i, o0, ow):
            def job():
                s0, w = dsplits[i]
                tw = pltpu.bitcast(wqkv_v[s0:s0 + w, o0:o0 + ow].T, U32)
                wqkv_w[o0 // 2:(o0 + ow) // 2, s0:s0 + w] = tw
                return [tw[-SUB:]] if w == LANES else []
            return job
        return [(1, tile(i, o0, ow)) for o0, ow in _lane_splits(3 * D) for i in range(len(dsplits))]

    def wo_jobs():
        def widen(i):
            def job():
                s0, w = dsplits[i]
                v = wo_v[:, s0:s0 + w].astype(F32)
                wo_f[i, 0:D, 0:w] = v
                return [_bits(v[-SUB:])] if w == LANES else []
            return job

        def regroup(d):
            def job():
                rows = [wo_f[i, pl.ds(d, H, stride=DH), :][:, 0:w] for i, (s0, w) in enumerate(dsplits)]
                pw = _words(jnp.concatenate(rows, axis=1))
                wo_p[d * SUB:(d + 1) * SUB, :] = pw
                return [pw[:, :LANES]]
            return job

        def turn(i, o0, ow):
            def job():
                s0, w = dsplits[i]
                tw = pltpu.bitcast(_halves(wo_p[s0 // 2:(s0 + w) // 2, o0:o0 + ow]).T, U32)
                wo_w[o0 // 2:(o0 + ow) // 2, s0:s0 + w] = tw
                return [tw[-SUB:]] if w == LANES else []
            return job

        return ([(2, widen(i)) for i in range(len(dsplits))] + [(1, regroup(d)) for d in range(DH)]
                + [(1, turn(i, o0, ow)) for i in range(len(dsplits)) for o0, ow in dsplits])

    N1 = 4 * LANES * LANES // T1
    U1 = F // N1

    def mix_units(c, lo, hi, jobs, first=False, h_cur=h_cur):
        sched.spread(jobs, [(i, rg) for i in range(lo, hi) for rg in range(D_RG)])
        for i in range(lo, hi):
            cols = slice(i * N1, (i + 1) * N1)
            lhs = sched.operand(i, lambda a, b: h_cur[a:b, :], D_RG)
            r = lax.dot_general(lhs, w1_v[_ds(c * T1, T1), cols], _NN, preferred_element_type=F32)
            u_f[:, cols] = r + (b1[:, cols] if first else u_f[:, cols])

    def next_norm_jobs(c, h_nxt=h_nxt):
        return [job for k in range(TPC) for job in norm_jobs((c + 1) * TPC + k, k, h_nxt)]

    cp_x(0).wait()
    for step in zip(*[norm_jobs(t, t, h_cur) for t in range(TPC)]):
        for _, job in step:
            job()
    cp_zero.wait()
    cp_b1.wait()
    cp_w1_head.wait()
    sched.zero = zero_v[...]
    b1 = b1_v[...].astype(F32).reshape(1, F)

    mix_units(0, 0, W1_HEAD // N1, [], first=True)
    cp_w1_rest.wait()
    cp_x(1).wait()
    mix_units(0, W1_HEAD // N1, U1, next_norm_jobs(0), first=True)
    h_cur[...] = h_nxt[...]

    def chunk(c, carry):
        cp_w1(c).wait()
        cp_x(c + 1).wait()

        sched.zero = zero_v[...]
        mix_units(c, 0, U1, next_norm_jobs(c))
        h_cur[...] = h_nxt[...]
        return carry

    lax.fori_loop(1, LOOPED + 1, chunk, 0)

    bufs = [h_cur, h_nxt]
    for c0 in range(LOOPED + 1, C1, PAIR):
        block = range(c0, min(C1, c0 + PAIR))
        for c in block:
            cp_w1(c).wait()
            if c + 1 < C1:
                cp_x(c + 1).wait()
            else:
                cp_wqkv.wait()
                cp_wo.wait()
                cp_b2.start()
                cp_w2.start()
        sched.zero = zero_v[...]
        for c in block:
            jobs = next_norm_jobs(c, bufs[1]) if c + 1 < C1 else wqkv_jobs()
            mix_units(c, 0, U1, jobs, h_cur=bufs[0])
            bufs.reverse()

    order2 = list(range(NT - HALO, NT)) + list(range(NT - HALO))

    def gelu_jobs(f):
        def job(rg):
            def run():
                gw = _words(_gelu(u_f[rg * RG:(rg + 1) * RG, f * LANES:(f + 1) * LANES]))
                g_w[rg * SUB:(rg + 1) * SUB, f * LANES:(f + 1) * LANES] = gw
                return [gw]
            return run
        return [(3, job(rg)) for rg in range(D_RG)]

    GAP = SKEW[4]
    HALF = D // 2

    def skew(ref, t):
        return SKEW[0] if ref is q_f else SKEW[1] if ref is k_f else SKEW[2 + t % 2]

    def put_tile(ref, t, val):
        o = skew(ref, t)
        ref[t, o:o + HALF, :] = val[:HALF]
        ref[t, o + HALF + GAP:o + D + GAP, :] = val[HALF:]

    def head_rows(ref, t, d):
        o = skew(ref, t) + d
        return jnp.concatenate([ref[t, pl.ds(o, H // 2, stride=DH), :],
                                ref[t, pl.ds(o + HALF + GAP, H // 2, stride=DH), :]], axis=0)

    def halo_jobs(j):
        src, dst = j + HALO, j + HALO - NT

        def job(ref, a, b):
            def run():
                gap = GAP if a >= HALF else 0
                r = pltpu.roll(ref[src, skew(ref, src) + gap + a:skew(ref, src) + gap + b, :], DIL, 1)
                ref[dst, skew(ref, dst) + gap + a:skew(ref, dst) + gap + b, :] = r
                return [_bits(r[i:i + SUB]) for i in range(0, b - a, 4 * SUB)]
            return run
        q = D // 4
        return [(4, job(ref, a, a + q)) for ref in (k_f, v_f) for a in range(0, D, q)]

    n_qkv_rg = 3 * D // RG
    gelu_all = [job for f in range(NF) for job in gelu_jobs(f)]
    per = -(-len(gelu_all) // 15)
    wo_prep = wo_jobs()
    for i, j in enumerate(order2):
        jobs = gelu_all[i * per:(i + 1) * per] if i < 15 else []
        if i >= 1 and order2[i - 1] >= NT - HALO:
            halo = halo_jobs(order2[i - 1])
            jobs = jobs[:len(jobs) // 2] + halo + jobs[len(jobs) // 2:]
        if i >= 9:
            k = -(-len(wo_prep) // 7)
            jobs = jobs + wo_prep[(i - 9) * k:(i - 8) * k]
        sched.spread(jobs, [(("p2", i), rg) for rg in range(n_qkv_rg)])

    for i, j in enumerate(order2):
        cols = [
            _halves(xn_tok[a, pl.ds(j, LANES // 2, stride=TOK_PITCH), :][:, 0:w])
            for a, (s0, w) in enumerate(dsplits)
        ]
        rows = jnp.concatenate(cols, axis=1)
        lhs = sched.operand(("p2", i), lambda a, b: wqkv_w[a:b, :], n_qkv_rg)
        r = lax.dot_general(lhs, rows, _NT, preferred_element_type=F32)
        put_tile(q_f, j, r[0:D])
        put_tile(k_f, j + HALO, r[D:2 * D])
        put_tile(v_f, j + HALO, r[2 * D:3 * D])

    lane = lax.broadcasted_iota(jnp.int32, (H, LANES), 1)

    def attention_jobs(j):
        st = {}

        def logits(w):
            def job():
                acc = None
                for d in range(DH):
                    t = head_rows(q_f, j, d) * head_rows(k_f, j + HALO - w, d)
                    acc = t if acc is None else acc + t
                acc = acc * scale
                if w > j:
                    acc = jnp.where(lane < DIL, -1e9, acc)
                st[w] = acc
                return [_bits(acc[:SUB]), _bits(acc[SUB:])]
            return job

        def softmax():
            mx = st[0]
            for w in range(1, W):
                mx = jnp.maximum(mx, st[w])
            e = [jnp.exp(st[w] - mx) for w in range(W)]
            den = e[0]
            for w in range(1, W):
                den = den + e[w]
            inv = 1.0 / den
            st["p"] = [e[w] * inv for w in range(W)]
            return [_bits(p[a:a + SUB]) for p in st["p"] for a in (0, SUB)]

        def values(d):
            def job():
                acc = None
                for w in range(W):
                    t = st["p"][w] * head_rows(v_f, j + HALO - w, d)
                    acc = t if acc is None else acc + t
                ow = _words(acc)
                o_w[j, d * SUB:(d + 1) * SUB, :] = ow
                return [ow]
            return job

        def scatter(i):
            def job():
                s0, w = dsplits[i]
                tw = pltpu.bitcast(_halves(o_w[j, s0 // 2:(s0 + w) // 2, :]).T, U32)
                o_tok[i, j * ATT_PITCH:j * ATT_PITCH + LANES // 2, 0:w] = tw
                return [tw[-SUB:]] if w == LANES else []
            return job

        core = [(110, logits(w)) for w in range(W)] + [(130, softmax)]
        core += [(32, values(d)) for d in range(DH)]
        return core, [(20, scatter(i)) for i in range(len(dsplits))]

    KG = 4 * LANES
    n_full, k_tail = F // KG, F % KG
    wide = KG // k_tail if k_tail else 1
    units3 = []
    for n0 in range(0, NT, wide):
        units3 += [(n, 1, g * KG, KG) for n in range(n0, n0 + wide) for g in range(n_full)]
        if k_tail:
            units3.append((n0, wide, n_full * KG, k_tail))
    n_att = ATT_TILES * len(units3) // NT

    def slots3(lo, hi):
        return [(("p3", u), rg) for u in range(lo, hi) for rg in range(D_RG)]

    att = [attention_jobs(j) for j in range(NT)]
    sched.spread([job for j in range(NT) for job in att[j][0]], slots3(0, n_att)[SKIP3:])
    sched.spread([job for j in range(NT) for job in att[j][1]], slots3(n_att, len(units3)))

    cp_b2.wait()
    cp_w2.wait()
    b2 = b2_v[...].astype(F32).reshape(1, S)
    for u, (n, nn, k0, kw) in enumerate(units3):
        ls = slice(n * LANES, (n + nn) * LANES)
        lhs = sched.operand(("p3", u), lambda a, b: g_w[a:b, k0:k0 + kw], D_RG)
        r = lax.dot_general(lhs, w2_v[k0:k0 + kw, ls], _NN, preferred_element_type=F32)
        if k0 == 0:
            y_f[:, ls] = r + b2[:, ls]
        else:
            y_f[:, ls] += r

    ends_out = {s0 + n: c for c, (s0, n) in enumerate(zip(starts_out, OUT_CHUNKS))}
    for n in range(NT):
        ls = slice(n * LANES, (n + 1) * LANES)
        cols = [
            jnp.concatenate(
                [_halves(o_tok[a, pl.ds(4 * n + q, NT, stride=ATT_PITCH), :][:, 0:w]) for q in range(4)], axis=0
            )
            for a, (s0, w) in enumerate(dsplits)
        ]
        o = jnp.concatenate(cols, axis=1)
        lhs = sched.operand(("p4", n), lambda a, b: wo_w[a:b, :], D_RG)
        a = lax.dot_general(lhs, o, _NT, preferred_element_type=F32)
        out_v[:, ls] = (x_v[:, ls].astype(F32) + a + y_f[:, ls]).astype(BF16)
        if (n + 1) * LANES in ends_out:
            cp_out[ends_out[(n + 1) * LANES]].start()
    assert not sched.plan, list(sched.plan)
    for cp in cp_out:
        cp.wait()


@jax.jit
def pallas_parallel_sum__sliding_local_dilated__mixer_token_mlp__prompt_kernel(
    A_x: jax.Array,
    A_wqkv: jax.Array,
    A_wo: jax.Array,
    B_x: jax.Array,
    B_w1: jax.Array,
    B_b1: jax.Array,
    B_w2: jax.Array,
    B_b2: jax.Array,
):
    del B_x
    Bsz, S, D = A_x.shape
    F = B_w1.shape[1]
    assert Bsz == 1 and S == 16 * LANES and D % H == 0 and D % (4 * RG) == 0 and F % LANES == 0
    assert (F % (4 * LANES)) in (0, LANES, 2 * LANES)
    assert S % T1 == 0 and S // T1 >= 5 and sum(OUT_CHUNKS) == S
    nct = -(-D // LANES)
    NT = S // LANES
    HALO = W - 1

    x_t = A_x.reshape(S, D).T

    def kern(*refs):
        _kernel(*refs, S=S, D=D, F=F)

    tile_rows = D + 4 * SUB
    hbm = pl.BlockSpec(memory_space=pl.ANY)
    scratch = [
        pltpu.VMEM((D, S), BF16),
        pltpu.VMEM((D, 3 * D), BF16),
        pltpu.VMEM((D, D), BF16),
        pltpu.VMEM((S, F), BF16),
        pltpu.VMEM((F, S), BF16),
        pltpu.VMEM((F,), BF16),
        pltpu.VMEM((S,), BF16),
        pltpu.VMEM((SUB, LANES), U32),
        pltpu.VMEM((SUB, LANES), U32),
        pltpu.VMEM((3 * D // 2, D), U32),
        pltpu.VMEM((nct, tile_rows, LANES), F32),
        pltpu.VMEM((D // 2, D), U32),
        pltpu.VMEM((D // 2, D), U32),
        pltpu.VMEM((T1 // LANES, D, LANES), F32),
        pltpu.VMEM((T1 // LANES, D // 2, LANES), U32),
        pltpu.VMEM((D // 2, T1), U32),
        pltpu.VMEM((D // 2, T1), U32),
        pltpu.VMEM((nct, (S // 32) * TOK_PITCH + 2 * SUB, LANES), U32),
        pltpu.VMEM((D, F), F32),
        pltpu.VMEM((D // 2, F), U32),
        pltpu.VMEM((NT, tile_rows, LANES), F32),
        pltpu.VMEM((NT + HALO, tile_rows, LANES), F32),
        pltpu.VMEM((NT + HALO, tile_rows, LANES), F32),
        pltpu.VMEM((NT, D // 2, LANES), U32),
        pltpu.VMEM((nct, (NT + 1) * ATT_PITCH - 2, LANES), U32),
        pltpu.VMEM((D, S), F32),
        pltpu.VMEM((D, S), BF16),
        pltpu.SemaphoreType.DMA((S // T1,)),
        pltpu.SemaphoreType.DMA((S // T1,)),
        pltpu.SemaphoreType.DMA((7,)),
        pltpu.SemaphoreType.DMA((len(OUT_CHUNKS),)),
    ]
    out_t = pl.pallas_call(
        kern,
        out_shape=jax.ShapeDtypeStruct((D, S), BF16),
        in_specs=[hbm] * 7,
        out_specs=hbm,
        scratch_shapes=scratch,
        compiler_params=pltpu.CompilerParams(vmem_limit_bytes=100 * 1024 * 1024),
    )(x_t, A_wqkv, A_wo, B_w1, B_w2, B_b1, B_b2)
    return out_t.T.reshape(1, S, D)
```
